```python
import os as _os
_os.environ.setdefault("JAX_PLATFORMS", "cpu")
import jax
import jax.numpy as jnp

def _softmax(x, axis=-1):
    return jax.nn.softmax(x, axis=axis)
def _gelu(x):
    return jax.nn.gelu(x, approximate=True)
def _silu(x):
    return jax.nn.silu(x)
def _sigmoid(x):
    return jax.nn.sigmoid(x)
def _layernorm(x, axis=-1, eps=1e-5):
    m = jnp.mean(x, axis=axis, keepdims=True)
    v = jnp.var(x, axis=axis, keepdims=True)
    return (x - m) / jnp.sqrt(v + eps)
def _scatter_add(tgt, idx, src, axis=0):
    return tgt.at[idx].add(src)
def _segment_sum(src, seg, n):
    return jax.ops.segment_sum(src, seg, n)
class _Rng:
    def __init__(self, key):
        self._k = key
    def _next(self):
        self._k, sub = jax.random.split(self._k)
        return sub
    def normal(self, shape):
        return jax.random.normal(self._next(), shape, dtype=jnp.bfloat16)
    def randint(self, lo, hi, shape):
        return jax.random.randint(self._next(), shape, lo, hi, dtype=jnp.int32)
    def uniform(self, shape, lo=0.0, hi=1.0):
        return jax.random.uniform(self._next(), shape, jnp.bfloat16, lo, hi)
    def permutation(self, n):
        return jax.random.permutation(self._next(), n)


kernel_name = 'concat_heads__linear_attn_block__ssm_conv_s4__prompt'

def setup_inputs():
    _rng = _Rng(jax.random.key(int.from_bytes(__import__("os").urandom(4), "little")))
    _w = (lambda a: (lambda t: t.astype(jnp.bfloat16) if jnp.issubdtype(t.dtype, jnp.floating) else t)(jnp.asarray(a)))
    def _A_setup():
        B, S, D = 1, 2048, 512
        return {
            "x": _w((lambda *s: _rng.normal(s) * 0.05)(B, S, D)),
            "wqkv": _w((lambda *s: _rng.normal(s) * 0.8)(D, 3 * D)),
            "wo": _w((lambda *s: _rng.normal(s) * 0.05)(D, D)),
        }
    _A_in = _A_setup()

    def _B_setup():
        B, L, D, N = 1, 2048, 512, 128
        A_re = -jnp.exp((lambda *s: _rng.normal(s) * 0.2)(D, N))
        A_im = jnp.pi * (lambda *s: _rng.normal(s) * 0.2)(D, N)
        B_re = (lambda *s: _rng.normal(s) * 0.2)(D, N)
        B_im = (lambda *s: _rng.normal(s) * 0.2)(D, N)
        C_re = (lambda *s: _rng.normal(s) * 0.2)(D, N)
        C_im = (lambda *s: _rng.normal(s) * 0.2)(D, N)
        log_dt = (lambda *s: _rng.normal(s) * 0.2)(D) * 0.5 - 4.0
        Dskip = (lambda *s: _rng.normal(s) * 0.05)(D)
        return {
            "u": _w((lambda *s: _rng.normal(s) * 0.05)(B, L, D)),
            "A_re": _w(A_re),
            "A_im": _w(A_im),
            "B_re": _w(B_re),
            "B_im": _w(B_im),
            "C_re": _w(C_re),
            "C_im": _w(C_im),
            "log_dt": _w(log_dt),
            "Dskip": _w(Dskip),
        }
    _B_in = _B_setup()

    return {
        "A_x": _A_in["x"],
        "A_wqkv": _A_in["wqkv"],
        "A_wo": _A_in["wo"],
        "B_u": _B_in["u"],
        "B_A_re": _B_in["A_re"],
        "B_A_im": _B_in["A_im"],
        "B_B_re": _B_in["B_re"],
        "B_B_im": _B_in["B_im"],
        "B_C_re": _B_in["C_re"],
        "B_C_im": _B_in["C_im"],
        "B_log_dt": _B_in["log_dt"],
        "B_Dskip": _B_in["Dskip"],
    }

def reference(A_x, A_wqkv, A_wo, B_u, B_A_re, B_A_im, B_B_re, B_B_im, B_C_re, B_C_im, B_log_dt, B_Dskip):
    def _A_ref(x, wqkv, wo):
        B, S, D = x.shape
        H = 32; Dh = D // H
        qkv = (lambda x, *d: x.transpose(*d))((x @ wqkv).reshape(B, S, 3, H, Dh), 2, 0, 3, 1, 4)
        q, k, v = qkv[0], qkv[1], qkv[2]
        phi = lambda t: jnp.where(t > 0, t + 1, jnp.exp(t)) + 1e-6
        pq, pk = phi(q), phi(k)
        kv = jnp.einsum("bhsd,bhse->bhde", pk, v)
        z = jnp.einsum("bhsd->bhd", pk)
        num = jnp.einsum("bhqd,bhde->bhqe", pq, kv)
        den = jnp.einsum("bhqd,bhd->bhq", pq, z)[..., None] + 1e-6
        o = num / den
        return (lambda x, *d: x.transpose(*d))(o, 0, 2, 1, 3).reshape(B, S, D) @ wo

    def _B_ref(u, A_re, A_im, B_re, B_im, C_re, C_im, log_dt, Dskip):
        Bsz, L, D = u.shape
        dt = jnp.exp(log_dt)[:, None]
        A = A_re + 1j * A_im
        Bc = B_re + 1j * B_im
        Cc = C_re + 1j * C_im
        logdA = dt * A
        dB = dt * Bc
        l = (lambda x, dt: x.astype(dt))(jnp.arange(L), A_re.dtype)
        P = jnp.exp(logdA[:, :, None] * l[None, None, :])
        K = jnp.einsum("dn,dnl,dn->dl", Cc, P, dB).real
        L2 = 2 * L
        Kp = jnp.pad(K, ((0, 0), (0, L)))
        up = (lambda x, *d: x.transpose(*d))(u, 0, 2, 1)
        up = jnp.pad(up, ((0, 0), (0, 0), (0, L)))
        Kf = (lambda x, axes=(-2,-1): jnp.fft.rfft2(x.astype(jnp.float32), axes=axes))(Kp[:, None, :], axes=(-2, -1))
        Uf = (lambda x, axes=(-2,-1): jnp.fft.rfft2(x.astype(jnp.float32), axes=axes))(up[:, :, None, :], axes=(-2, -1))
        Yf = Uf * Kf[None, :, :, :]
        y = (lambda x, s, axes=(-2,-1): jnp.fft.irfft2(x, s=s, axes=axes).astype(jnp.bfloat16))(Yf, (1, L2), axes=(-2, -1))[:, :, 0, :L]
        y = (lambda x, *d: x.transpose(*d))(y, 0, 2, 1) + u * Dskip[None, None, :]
        return y

    a = _A_ref(A_x, A_wqkv, A_wo)
    b = _B_ref(B_u, B_A_re, B_A_im, B_B_re, B_B_im, B_C_re, B_C_im, B_log_dt, B_Dskip)
    return jnp.concatenate([a, b], axis=-1)
```

```python
import functools

import jax
import jax.numpy as jnp
import ml_dtypes
import numpy as np
from jax import lax
import jax.experimental.pallas as pl
import jax.experimental.pallas.tpu as pltpu

F32, BF16, U32, I32 = jnp.float32, jnp.bfloat16, jnp.uint32, jnp.int32

L = 2048
D = 512
N = 128
CH = 256
NC = L // CH
NN = (((1,), (0,)), ((), ()))
NT = (((1,), (1,)), ((), ()))
TN = (((0,), (0,)), ((), ()))

_OFF = ((0, 1, 2, 3), (4, 5, 6, 7), (256, 258, 260, 262), (512, 516, 768, 772),
        (1024, 1280, 1536, 1792))
_TILES = ((0, 1), (2,), (3,), (3,), (4,), (4,), (4,), (4,))
_FIX = {1: 512, 3: 1024, 7: 2048}


@functools.cache
def _constants():
    bf = ml_dtypes.bfloat16
    lq = np.arange(L).astype(np.float32).astype(bf).astype(np.int64)
    f = np.concatenate([np.arange(0, CH, 2), np.arange(1, CH, 2)])
    om = 2 * np.pi * (f + 0.5) / (2 * CH)
    s = np.arange(128)
    cf = np.cos(om[:, None] * (s + 0.5))
    sf = -np.sin(om[:, None] * (s + 0.5))
    rows = np.array([16 * k + 2 * r + p for k in range(8) for p in range(2) for r in range(8)])
    at = cf.T[rows] / CH
    bt = sf.T[rows] / CH

    def lanemap(tau):
        h = tau & 1 if tau < 4 else 0
        val = np.zeros(128, np.int64)
        for kap in range(4):
            for j in range(32):
                val[(32 * (j >> 3) + (j & 7) + 24 + 8 * kap + 4 * h) % 128] = _OFF[tau][kap] + 8 * j
        return val

    def wmat(m, vals):
        ph = np.exp(-1j * om[:, None] * np.arange(CH)[None, :])
        sel = (lq[CH * m:CH * (m + 1), None] == vals[None, :]).astype(np.float64)
        w = ph @ sel
        return np.concatenate([w.real, w.imag], 0)

    fwd = np.concatenate([cf, sf], 0)
    inv = np.concatenate([at[:, :128], at[:, 128:], bt[:, :128], bt[:, 128:]], 0)
    wk = np.concatenate([wmat(m, lanemap(t)) for m in range(NC) for t in _TILES[m]], 0)
    perm = np.zeros((128, 128))
    for d in range(16):
        for hl in range(8):
            perm[8 * d + hl, 16 * hl + d] = 1.0
    phi = np.concatenate([np.broadcast_to(wmat(m, np.array([v])), (2 * CH, 128)) for m, v in _FIX.items()], 0)
    return (fwd.astype(bf), inv.astype(bf), wk.astype(bf), perm.astype(bf), phi.astype(np.float32))


def _bf(v):
    return pltpu.bitcast(v, BF16)


def _w(v):
    return pltpu.bitcast(v, U32)


def _pack(a, b):
    return pltpu.pack_elementwise([a, b], packed_dtype=BF16)


def _unpack(v, i):
    return pltpu.unpack_elementwise(v, index=i, packed_dtype=BF16, unpacked_dtype=F32)


def _dot(a, b, dims=NN):
    return lax.dot_general(a, b, dims, preferred_element_type=F32)


def _cmul(a, b):
    return a[0] * b[0] - a[1] * b[1], a[0] * b[1] + a[1] * b[0]


def _csq(a):
    t = a[0] * a[1]
    return a[0] * a[0] - a[1] * a[1], t + t


def _phi(t):
    return jnp.where(t > 0, t + 1.0, jnp.exp(t)) + 1e-6


def _cexp(re, im):
    t = im * np.float32(1.0 / (2.0 * np.pi))
    magic = np.float32(1.5 * 2.0 ** 23)
    fr = t - ((t + magic) - magic)
    x = fr * np.float32(np.pi / 2.0)
    z = x * x
    sn = x + x * z * (np.float32(-1.6666654611e-1) + z * (np.float32(8.3321608736e-3) + z * np.float32(-1.9515295891e-4)))
    cs = 1.0 + z * (np.float32(-0.5) + z * (np.float32(4.166664568298827e-2) + z * (np.float32(-1.388731625493765e-3) + z * np.float32(2.443315711809948e-5))))
    r = jnp.exp(re * 0.25)
    return _csq(_csq((r * cs, r * sn)))


def _kernel(x_h, wqkv_h, wo_h, u_h, are_h, aim_h, bre_h, bim_h, cre_h, cim_h, ldt_h, dsk_h,
            fwd_h, inv_h, wk_h, perm_h, phi_h,
            out_h,
            xs, wq, wk, wv, wo, us, par, small, fwd, inv, wm, perm, phi,
            wqt, gt, mm, zb, dtb, jbuf, kd, xsp, kh, uh, zz, ob, oa, sems, osems):
    hu = lambda r: r.bitcast(U32)
    copies = {}

    def dma(name, src, dst):
        copies[name] = pltpu.make_async_copy(src, dst, sems.at[len(copies)])
        copies[name].start()

    def wait(*names):
        for n in names:
            copies[n].wait()

    dma("ldt", ldt_h, small.at[0])
    for i, r in enumerate((are_h, aim_h, bre_h, bim_h, cre_h, cim_h)):
        dma(f"par{i}", hu(r), par.at[i])
    dma("wk", hu(wqkv_h).at[:, pl.ds(D, D)], wk)
    dma("x", hu(x_h), xs)
    dma("fwd", hu(fwd_h), fwd)
    for b in range(4):
        dma(f"u{b}", hu(u_h).at[:, pl.ds(128 * b, 128)], us.at[b])
    dma("wm", hu(wk_h), wm)
    dma("dsk", dsk_h, small.at[1])
    dma("phi", phi_h, phi)
    dma("inv", hu(inv_h), inv)
    dma("perm", hu(perm_h), perm)
    dma("wq", hu(wqkv_h).at[:, pl.ds(0, D)], wq)
    dma("wv", hu(wqkv_h).at[:, pl.ds(2 * D, D)], wv)
    dma("wo", hu(wo_h), wo)
    wait(*copies)

    sub = lax.broadcasted_iota(I32, (8, 128), 0)
    lane = lax.broadcasted_iota(I32, (8, 128), 1)
    odd = sub & 1
    kap = ((lane + (104 - 4 * odd)) >> 3)
    bit0 = (kap & 1) != 0
    bit1 = (kap & 2) != 0
    bit0e = (((lane + 104) >> 3) & 1) != 0
    low = sub < 4
    rev8 = 7 - sub
    rev4 = sub ^ 3
    perm8 = lambda v, idx: jnp.take_along_axis(v, idx, axis=0)

    def dt_table(b):
        dt = jnp.exp(small[0].astype(F32)).astype(BF16).astype(F32)
        dtb[...] = jnp.broadcast_to(dt[b:b + 1, :], (128, 128)).T

    def gen_unit(b, un):
        rows = pl.ds(64 * b + 8 * un, 8)
        words = [par[i, rows, :] for i in range(6)]
        lhs, special = [], []
        for g in range(2):
            are, aim, bre, bim, cre, cim = [_unpack(v, g) for v in words]
            dt = dtb[pl.ds(16 * un + g, 8, stride=2), :]
            a1 = _cexp(dt * are, dt * aim)
            a8 = _csq(_csq(_csq(a1)))
            a8 = (perm8(a8[0], rev4), perm8(a8[1], rev4))
            a16 = _csq(a8)
            e = (jnp.ones_like(dt), jnp.zeros_like(dt))
            o = a8
            for k in range(16):
                dst = pl.ds(32 * (k >> 2) + (k & 3), 8, stride=4)
                for c in range(2):
                    jbuf[un, g, c, dst, :] = _pack(e[c], o[c])
                e = a16 if k == 0 else _cmul(e, a16)
                if k < 15:
                    o = _cmul(o, a16)
            a1c = (a1[0], -a1[1])
            a256c = (perm8(e[0], rev4), -perm8(e[1], rev4))
            cb = _cmul((cre, cim), (bre, bim))
            v = [(cb[0] * dt, -(cb[1] * dt))]
            for r in range(7):
                v.append(_cmul(v[-1], a1c))
            t2 = [_cmul(v[2 * k], a256c) for k in range(4)]
            t3 = [_cmul(t2[0], a256c), _cmul(t2[2], a256c)]
            t3 += [_cmul(t3[0], a256c), _cmul(t3[1], a256c)]
            t4 = [_cmul(t3[2], a256c)]
            for k in range(3):
                t4.append(_cmul(t4[-1], a256c))
            special.append((t3[0][0], t4[0][0], t4[3][0] * a256c[0] - t4[3][1] * a256c[1]))
            quads = [[], []]
            for c in range(2):
                pairs = [(_pack(v[k][c], v[4 + k][c]), _pack(t2[k][c], t3[k][c])) for k in range(4)]
                pairs.append((_pack(t4[0][c], t4[1][c]), _pack(t4[2][c], t4[3][c])))
                q0, q1 = [], []
                for p, r in pairs:
                    r4 = pltpu.roll(r, 4, 0)
                    q0.append(jnp.where(low, p, r4))
                    q1.append(jnp.where(low, r4, p))
                quads[0].append(jnp.concatenate(q0, 0))
                quads[1].append(jnp.concatenate(q1, 0))
            lhs.append([_bf(jnp.concatenate(q, 1)) for q in quads])
        for s in range(3):
            xsp[s, pl.ds(8 * un, 8), :] = _pack(special[0][s], special[1][s])
        for q in range(2):
            merged = []
            for g in range(2):
                rhs = jnp.concatenate([
                    jnp.concatenate([jbuf[un, g, c, pl.ds(32 * jj + 16 * q, 16), :] for jj in range(4)], 0)
                    for c in range(2)], 1)
                res = _dot(lhs[g][q], _bf(rhs), NT)
                vr = lambda i, h: res[16 * i + 8 * (h ^ q):16 * i + 8 * (h ^ q) + 8]
                rot = lambda v, k: pltpu.roll(v, 8 * k, 1, stride=4, stride_axis=0)
                ms = []
                for h in range(2):
                    r = [rot(vr(k, h), k) for k in range(4)]
                    ms.append(jnp.where(bit1, jnp.where(bit0, r[3], r[2]), jnp.where(bit0, r[1], r[0])))
                t = jnp.where(bit1, rot(vr(4, 1), 2), rot(vr(4, 0), 0))
                ms.append(jnp.where(odd != 0, pltpu.roll(t, 4, 1), t))
                merged.append(ms)
            for i in range(3):
                kd[i, pl.ds(16 * un + 8 * q, 8), :] = _pack(merged[0][i], merged[1][i])

    def ktile(t):
        ld = lambda i, h: jnp.concatenate([kd[i, pl.ds(16 * un + h, 8, stride=2), :] for un in range(8)], 0)
        if t < 4:
            return _bf(ld(t >> 1, t & 1))
        m = jnp.concatenate([bit0e] * 8, 0)
        return _bf(jnp.where(m, ld(2, 1), ld(2, 0)))

    def khat(b):
        idx = 0
        ones = jnp.ones((16, 128), BF16)
        for m in range(NC):
            acc = None
            for t in _TILES[m]:
                r = _dot(_bf(wm[pl.ds(256 * idx, 256), :]), ktile(t), NT)
                acc = r if acc is None else acc + r
                idx += 1
            if m in _FIX:
                s = list(_FIX).index(m)
                sp = _dot(ones, _bf(xsp[s]), NT)[0:1]
                acc = acc + phi[pl.ds(2 * CH * s, 2 * CH), :] * sp
            if m == 0:
                dsk = small[1].astype(F32)[b:b + 1, :]
                kh[0, pl.ds(0, CH), :] = acc[:CH] + dsk
                kh[0, pl.ds(CH, CH), :] = acc[CH:]
            else:
                kh[m] = acc

    def uhat(b, c):
        ev, od = [], []
        for k in range(8):
            wu = us[b, pl.ds(128 * c + 64 + 8 * k, 8), :]
            wl = perm8(us[b, pl.ds(128 * c + 56 - 8 * k, 8), :], rev8)
            u0, u1, l0, l1 = _unpack(wu, 0), _unpack(wu, 1), _unpack(wl, 0), _unpack(wl, 1)
            ev.append(_pack(u0 + l1, u1 + l0))
            od.append(_pack(u0 - l1, u1 - l0))
        uh[c, pl.ds(0, CH), :] = _dot(_bf(fwd[pl.ds(0, 128), :]), _bf(jnp.concatenate(ev, 0)))
        uh[c, pl.ds(CH, CH), :] = _dot(_bf(fwd[pl.ds(128, 128), :]), _bf(jnp.concatenate(od, 0)))

    def conv_rows(r):
        res = []
        for hh in range(2):
            row = 16 * r + 8 * hh
            kr = [kh[j, pl.ds(row, 8), :] for j in range(NC)]
            ki = [kh[j, pl.ds(CH + row, 8), :] for j in range(NC)]
            ur = [uh[j, pl.ds(row, 8), :] for j in range(NC)]
            ui = [uh[j, pl.ds(CH + row, 8), :] for j in range(NC)]
            if row < 128:
                tr = [ur[0]] + [ur[c] - ui[c - 1] for c in range(1, NC)]
                ti = [ui[0]] + [ui[c] + ur[c - 1] for c in range(1, NC)]
            else:
                tr = [ur[0]] + [ur[c] + ui[c - 1] for c in range(1, NC)]
                ti = [ui[0]] + [ui[c] - ur[c - 1] for c in range(1, NC)]
            ks = [a + b for a, b in zip(kr, ki)]
            ts = [a + b for a, b in zip(tr, ti)]
            out = []
            for c in range(NC):
                p = [functools.reduce(lambda a, b: a + b, [x[j] * y[c - j] for j in range(c + 1)])
                     for x, y in ((kr, tr), (ki, ti), (ks, ts))]
                out.append((p[0] - p[1], p[2] - p[0] - p[1]))
            res.append(out)
        for c in range(NC):
            for comp in range(2):
                v = jnp.concatenate([res[0][c][comp], res[1][c][comp]], 0).astype(BF16)
                zz[c, pl.ds(128 * comp + 8 * r, 8), :] = _w(v)

    def inverse(b, c):
        lhs = lambda i: _bf(jnp.concatenate([inv[pl.ds(128 * i, 64), :], inv[pl.ds(128 * i + 64, 64), :]], 1))
        av = _dot(lhs(0), _bf(zz[c, pl.ds(0, 128), :]))
        bv = _dot(lhs(1), _bf(zz[c, pl.ds(128, 128), :]))
        up, dn = av + bv, av - bv
        for k in range(8):
            e, o = slice(16 * k, 16 * k + 8), slice(16 * k + 8, 16 * k + 16)
            ob[b, pl.ds(128 * c + 64 + 8 * k, 8), :] = _pack(up[e], up[o])
            ob[b, pl.ds(128 * c + 56 - 8 * k, 8), :] = perm8(_pack(dn[o], dn[e]), rev8)

    outs = []

    def out_dma(src, dst):
        c = pltpu.make_async_copy(src, dst, osems.at[len(outs)])
        c.start()
        outs.append(c)

    TT = 512
    zacc = jnp.zeros((8, D), F32)
    for t in range(L // TT):
        xt = _bf(xs[pl.ds(TT // 2 * t, TT // 2), :])
        pk = _phi(_dot(xt, _bf(wk[...])))
        zacc = zacc + pk.reshape(TT // 8, 8, D).sum(0)
        g = _dot(xt, pk.astype(BF16), TN)
        gt[...] = g if t == 0 else gt[...] + g
    z = zacc.sum(0, keepdims=True).astype(BF16)
    pm = _bf(perm[...])
    r128 = lax.broadcasted_iota(I32, (128, 128), 0)
    c128 = lax.broadcasted_iota(I32, (128, 128), 1)
    same_head = (r128 >> 4) == (c128 >> 4)
    for b in range(4):
        cols = pl.ds(128 * b, 128)
        kv = _dot(gt[:, cols].astype(BF16), _bf(wv[:, cols]), TN)
        kv = jnp.where(same_head, kv, 0.0).astype(BF16)
        kvp = _dot(pm, kv).astype(BF16)
        mm[pl.ds(64 * b, 64), :] = _w(_dot(kvp, _bf(wo[pl.ds(64 * b, 64), :])).astype(BF16))
        zb[pl.ds(128 * b, 128), :] = _dot(pm, jnp.broadcast_to(z[:, 128 * b:128 * b + 128], (128, 128)), NT)
        wqt[pl.ds(64 * b, 64), :] = _w(_dot(pm, _bf(wq[:, cols]), NT).astype(BF16))
    for t in range(L // TT):
        xt = _bf(xs[pl.ds(TT // 2 * t, TT // 2), :])
        pq = _phi(_dot(_bf(wqt[...]), xt, NT))
        pn = []
        for b in range(4):
            blk = [pq[128 * b + 8 * d:128 * b + 8 * d + 8] for d in range(16)]
            zs = [jnp.concatenate([zb[pl.ds(128 * b + 8 * d, 8), :]] * (TT // 128), 1) for d in range(16)]
            den = functools.reduce(lambda a, c: a + c, [p * zv for p, zv in zip(blk, zs)]) + 1e-6
            rd = 1.0 / den
            pn += [p * rd for p in blk]
        o = _dot(jnp.concatenate(pn, 0).astype(BF16), _bf(mm[...]), TN)
        oa[pl.ds(TT // 2 * t, TT // 2), :] = _w(o.astype(BF16))
        out_dma(oa.at[pl.ds(TT // 2 * t, TT // 2), :], hu(out_h).at[pl.ds(TT // 2 * t, TT // 2), pl.ds(0, D)])

    for b in range(4):
        dt_table(b)
        for un in range(8):
            gen_unit(b, un)
        khat(b)
        for c in range(NC):
            uhat(b, c)
        for r in range(16):
            conv_rows(r)
        for c in range(NC):
            inverse(b, c)
        out_dma(ob.at[b], hu(out_h).at[:, pl.ds(D + 128 * b, 128)])
    for c in outs:
        c.wait()


@jax.jit
def pallas_concat_heads__linear_attn_block__ssm_conv_s4__prompt_kernel(A_x, A_wqkv, A_wo, B_u, B_A_re, B_A_im, B_B_re, B_B_im, B_C_re, B_C_im, B_log_dt, B_Dskip):
    consts = _constants()
    ins = (A_x.reshape(L, D), A_wqkv, A_wo, B_u.reshape(L, D), B_A_re, B_A_im, B_B_re, B_B_im,
           B_C_re, B_C_im, B_log_dt.reshape(4, 128), B_Dskip.reshape(4, 128)) + consts
    vm = pltpu.VMEM
    scratch = [
        vm((L // 2, D), U32), vm((D // 2, D), U32), vm((D // 2, D), U32), vm((D // 2, D), U32), vm((D // 2, D), U32),
        vm((4, L // 2, 128), U32), vm((6, D // 2, N), U32), vm((2, 4, 128), BF16),
        vm((256, 128), U32), vm((256, 128), U32), vm((9 * 256, 128), U32), vm((64, 128), U32), vm((3 * 512, 128), F32),
        vm((D // 2, D), U32), vm((D, D), F32), vm((D // 2, D), U32), vm((D, 128), F32), vm((128, 128), F32),
        vm((8, 2, 2, 128, 128), U32), vm((3, 128, 128), U32), vm((3, 64, 128), U32),
        vm((NC, 512, 128), F32), vm((NC, 512, 128), F32), vm((NC, 256, 128), U32),
        vm((4, L // 2, 128), U32), vm((L // 2, D), U32),
        pltpu.SemaphoreType.DMA((32,)), pltpu.SemaphoreType.DMA((32,)),
    ]
    out = pl.pallas_call(
        _kernel,
        out_shape=jax.ShapeDtypeStruct((L, 2 * D), BF16),
        in_specs=[pl.BlockSpec(memory_space=pl.ANY)] * len(ins),
        out_specs=pl.BlockSpec(memory_space=pl.ANY),
        scratch_shapes=scratch,
        compiler_params=pltpu.CompilerParams(vmem_limit_bytes=100 * 2 ** 20),
        name="fused_k",
    )(*ins)
    return out.reshape(1, L, 2 * D)
```

```python
import functools
import os

import jax
import jax.numpy as jnp
import ml_dtypes
import numpy as np
from jax import lax
import jax.experimental.pallas as pl
import jax.experimental.pallas.tpu as pltpu

F32, BF16, U32, I32 = jnp.float32, jnp.bfloat16, jnp.uint32, jnp.int32

L = 2048
D = 512
N = 128
CH = 256
NC = L // CH
NZ = 16
NN = (((1,), (0,)), ((), ()))
NT = (((1,), (1,)), ((), ()))

CFG = dict(u0=10, wgt=150, pinkd=0, gauss=0, split=40, tb=0, skip=0, pstep=3, gen_a0=15, gen_a=12, gen_a2=11, kh_a=3, look=2, ahead=0, pinb=1, pink=1, jstep=1, tail=9, pre=2, e0=64, e1=122, e2=183)
for kv in os.environ.get("KCFG", "").split(","):
    if kv:
        k_, v_ = kv.split("=")
        CFG[k_] = int(v_)

_OFF = ((0, 1, 2, 3), (4, 5, 6, 7), (256, 258, 260, 262), (512, 516, 768, 772),
        (1024, 1280, 1536, 1792))
_TILES = ((0, 1), (2,), (3,), (3,), (4,), (4,), (4,), (4,))
_FIX = {1: 512, 3: 1024, 7: 2048}


@functools.cache
def _constants():
    bf = ml_dtypes.bfloat16
    lq = np.arange(L).astype(np.float32).astype(bf).astype(np.int64)
    f = np.concatenate([np.arange(0, CH, 2), np.arange(1, CH, 2)])
    om = 2 * np.pi * (f + 0.5) / (2 * CH)
    s = np.arange(128)
    cf = np.cos(om[:, None] * (s + 0.5))
    sf = -np.sin(om[:, None] * (s + 0.5))
    rows = np.array([16 * k + 2 * r + p for k in range(8) for p in range(2) for r in range(8)])
    at = cf.T[rows] / CH
    bt = sf.T[rows] / CH

    def lanemap(tau):
        h = tau & 1 if tau < 4 else 0
        val = np.zeros(128, np.int64)
        for kap in range(4):
            for j in range(32):
                val[(32 * (j >> 3) + (j & 7) + 24 + 8 * kap + 4 * h) % 128] = _OFF[tau][kap] + 8 * j
        return val

    def wmat(m, vals):
        ph = np.exp(-1j * om[:, None] * np.arange(CH)[None, :])
        sel = (lq[CH * m:CH * (m + 1), None] == vals[None, :]).astype(np.float64)
        w = ph @ sel
        return np.concatenate([w.real, w.imag], 0)

    fwd = np.concatenate([cf, sf], 0)
    inv = np.concatenate([at[:, :128], at[:, 128:], bt[:, :128], bt[:, 128:]], 0)
    wk = np.concatenate([wmat(m, lanemap(t)) for m in range(NC) for t in _TILES[m]], 0)
    phi = np.zeros((8, 2 * CH))
    for i, (m, v) in enumerate(_FIX.items()):
        phi[i] = wmat(m, np.array([v]))[:, 0]
    zero = np.zeros((2 * NZ,), np.int32)
    zero[NZ:] = 1
    return (fwd.astype(bf), inv.astype(bf), wk.astype(bf), phi.astype(np.float32), zero)


def _bf(v):
    return pltpu.bitcast(v, BF16)


def _w(v):
    return pltpu.bitcast(v, U32)


def _pack(a, b):
    return pltpu.pack_elementwise([a, b], packed_dtype=BF16)


def _unpack(v, i):
    return pltpu.unpack_elementwise(v, index=i, packed_dtype=BF16, unpacked_dtype=F32)


def _dot(a, b, dims=NN):
    return lax.dot_general(a, b, dims, preferred_element_type=F32)


def _cmul(a, b):
    return a[0] * b[0] - a[1] * b[1], a[0] * b[1] + a[1] * b[0]


def _csq(a):
    t = a[0] * a[1]
    return a[0] * a[0] - a[1] * a[1], t + t


def _phi(t):
    return jnp.where(t > 0, t + 1.0, jnp.exp(t)) + 1e-6


def _sum(xs):
    return functools.reduce(lambda a, b: a + b, xs)


def _kernel(x_h, wqkv_h, wo_h, u_h, are_h, aim_h, bre_h, bim_h, cre_h, cim_h, ldt_h, dsk_h,
            fwd_h, inv_h, wk_h, phi_h, zero_h,
            out_h,
            xs, wq, wk, wv, wo, us, par, ldt, dsk, fwd, inv, wm, phi,
            wqt, gt0, gt1, gt2, gt3, mm, zb, zt, jbuf, kd, xsp, kh, uh, zz, ob, oa,
            pk0, pk1, pq0, pq1, pq2, phit, zs, sems):
    hu = lambda r: r.bitcast(U32)
    batches = {}

    def dma(batch, src, dst):
        if batch not in batches:
            batches[batch] = (len(batches), [])
        c = pltpu.make_async_copy(src, dst, sems.at[batches[batch][0]])
        c.start()
        batches[batch][1].append(c)

    def wait(*names):
        for n in names:
            for c in batches[n][1]:
                c.wait()
            batches[n][1].clear()

    pars = (are_h, aim_h, bre_h, bim_h, cre_h, cim_h)

    def x_dma(batch, r0, n):
        for j in range(4):
            dma(batch, hu(x_h).at[pl.ds(r0 // 2, n // 2), pl.ds(128 * j, 128)], xs.at[j, pl.ds(r0 // 2, n // 2), :])

    def col_dma(batch, src, c0, dst):
        dma(batch, hu(src).at[:, pl.ds(c0, 128)], dst)

    def par_dma(batch, b0, nb):
        for i, r in enumerate(pars):
            rows = pl.ds(64 * b0, 64 * nb)
            dma(batch, hu(r).at[rows, :], par.at[i, rows, :])

    dma("a", zero_h, zs)
    dma("a", hu(ldt_h), ldt)
    dma("a", phi_h, phi)
    par_dma("a", 0, 1)
    col_dma("a", wqkv_h, D, wk.at[0])
    x_dma("a", 0, 128)
    for i in range(1, 4):
        x_dma(("x", i), 128 * i, 128)
    col_dma(("wk", 1), wqkv_h, D + 128, wk.at[1])
    col_dma(("wk", 2), wqkv_h, D + 256, wk.at[2])
    dma(("wk", 2), hu(fwd_h), fwd)
    col_dma(("wk", 2), u_h, 0, us.at[0])
    col_dma(("wk", 3), wqkv_h, D + 384, wk.at[3])
    dma("wm", dsk_h, dsk)
    dma("wm", hu(wk_h), wm)
    par_dma("c0", 1, 1)
    x_dma("c0", 512, 512)
    x_dma("g1", 1024, 1024)
    dma("g1", hu(inv_h), inv)
    col_dma("g1", u_h, 128, us.at[1])
    par_dma("g1", 2, 2)
    for b in range(4):
        col_dma("g1", wqkv_h, 128 * b, wq.at[b])
    for b in range(2, 4):
        col_dma("rest", u_h, 128 * b, us.at[b])
    for b in range(4):
        col_dma("rest", wqkv_h, 2 * D + 128 * b, wv.at[b])
    for b in range(4):
        col_dma("rest", wo_h, 128 * b, wo.at[b])

    wait("a")
    zoff = [zs[i] for i in range(NZ)]

    def ds(start, size, tag):
        return pl.ds(pl.multiple_of(zoff[tag % NZ] + start, 8), size)

    def xrows(tok0, n, tag):
        return jnp.concatenate([xs[j, ds(tok0 // 2, n // 2, tag), :] for j in range(4)], 1)

    sub = lax.broadcasted_iota(I32, (8, 128), 0)
    lane = lax.broadcasted_iota(I32, (8, 128), 1)
    odd = sub & 1
    kap = ((lane + (104 - 4 * odd)) >> 3)
    bit0 = (kap & 1) != 0
    bit1 = (kap & 2) != 0
    bit0e = (((lane + 104) >> 3) & 1) != 0
    low = sub < 4
    rev8 = 7 - sub
    rev4 = sub ^ 3
    always = (lane * sub) >= 0
    perm8 = lambda v, idx: jnp.take_along_axis(v, idx, axis=0)

    pins = []
    credit = [0.0, 0.0, 1.0]

    def pin(v, cost):
        pins.append((_w(v), cost))

    def pinned(words):
        if not pins:
            credit[1] = 0.0
            return words
        rows = []
        for i in range(words.shape[0] // 8):
            row = []
            for j in range(words.shape[1] // 128):
                v = words[8 * i:8 * i + 8, 128 * j:128 * j + 128]
                credit[1] += credit[0] * credit[2]
                if pins and credit[1] >= pins[0][1]:
                    tok, cost = pins.pop(0)
                    credit[1] -= cost
                    v = jnp.where(always, v, tok)
                row.append(v)
            rows.append(jnp.concatenate(row, 1) if len(row) > 1 else row[0])
        return jnp.concatenate(rows, 0)

    late = []

    def pinned_rhs(words):
        if not late:
            return words
        v = [words[8 * i:8 * i + 8] for i in range(32)]
        for j in range(4):
            if late:
                v[8 * j + 7] = jnp.where(always, v[8 * j + 7], late.pop(0))
        return jnp.concatenate(v, 0)

    def pinned4(ws):
        v = pinned(jnp.concatenate(ws, 1)) if CFG["pinb"] else jnp.concatenate(ws, 1)
        return [_bf(v[:, 128 * p:128 * p + 128]) for p in range(4)]

    def drain_over(units, extra=0.0):
        kinds = [last[0]] + [e[2] for e in au]
        total = sum([WEIGHT[k] for k, cur in zip(kinds, kinds[1:]) if cur != "n"][:units]) + extra
        credit[0] = 1.03 * sum(c for _, c in pins) / (32.0 * max(total, 0.5))

    last = ["b"]
    w = CFG["wgt"] / 100.0
    WEIGHT = dict(k=1 - 0.2 * w, g=1 + 0.2 * w, q=1 - 0.45 * w, o=1 + 0.3 * w, b=1.0, n=1.3)

    def begin(kind):
        credit[2] = WEIGHT[last[0]]
        last[0] = kind

    held = {}

    def gen_vpu(b, gi):
        un, g = divmod(gi, 2)
        rows = pl.ds(64 * b + 8 * un, 8)
        are, aim, bre, bim, cre, cim = [_unpack(par[i, rows, :], g) for i in range(6)]
        dt = [jnp.full((8, 128), ldt[b // 2, 16 * un + 2 * i + g], U32) for i in range(8)]
        for m in (odd != 0, (sub & 2) != 0, sub >= 4):
            dt = [jnp.where(m, dt[i + 1], dt[i]) for i in range(0, len(dt), 2)]
        pin(dt[0], 15)
        dt = jnp.exp(_unpack(dt[0], b % 2)).astype(BF16).astype(F32)
        pin(dt, 10)
        t = (dt * aim) * np.float32(1.0 / (2.0 * np.pi))
        magic = np.float32(1.5 * 2.0 ** 23)
        x = (t - ((t + magic) - magic)) * np.float32(np.pi / 2.0)
        z = x * x
        pin(z, 9)
        sn = x + x * z * (np.float32(-1.6666654611e-1) + z * (np.float32(8.3321608736e-3) + z * np.float32(-1.9515295891e-4)))
        cs = 1.0 + z * (np.float32(-0.5) + z * (np.float32(4.166664568298827e-2) + z * (np.float32(-1.388731625493765e-3) + z * np.float32(2.443315711809948e-5))))
        r = jnp.exp((dt * are) * 0.25)
        a1 = (r * cs, r * sn)
        pin(cs, 12)
        pin(a1[0], 8)
        pin(a1[1], 8)
        for i in range(5):
            a1 = _csq(a1)
            if i == 1:
                a1c = (a1[0], -a1[1])
            if i in (1, 4):
                pin(a1[0], 12)
        a8 = (perm8(a1[0], rev4), perm8(a1[1], rev4))
        a16 = _csq(a8)
        e = (jnp.ones_like(dt), jnp.zeros_like(dt))
        o = a8
        for k in range(16):
            dst = pl.ds(32 * (k >> 2) + (k & 3), 8, stride=4)
            for c in range(2):
                wd = _pack(e[c], o[c])
                jbuf[gi, c, dst, :] = wd
                if k % CFG["jstep"] == CFG["jstep"] - 1:
                    pin(wd, 7 * CFG["jstep"])
            e = a16 if k == 0 else _cmul(e, a16)
            if k < 15:
                o = _cmul(o, a16)
        a256c = (perm8(e[0], rev4), -perm8(e[1], rev4))
        cb = _cmul((cre, cim), (bre, bim))
        v = [(cb[0] * dt, -(cb[1] * dt))]
        for r in range(7):
            v.append(_cmul(v[-1], a1c))
            if r % 2 == 0:
                pin(v[-1][0], 12)
        t2 = [_cmul(v[2 * k], a256c) for k in range(4)]
        t3 = [_cmul(t2[0], a256c), _cmul(t2[2], a256c)]
        t3 += [_cmul(t3[0], a256c), _cmul(t3[1], a256c)]
        t4 = [_cmul(t3[2], a256c)]
        for k in range(3):
            t4.append(_cmul(t4[-1], a256c))
        late = {1: t3[2][0], 2: t4[0][0], 3: t4[2][0]}
        special = (t3[0][0], t4[0][0], t4[3][0] * a256c[0] - t4[3][1] * a256c[1])
        quads = [[[], []], [[], []]]
        for k in range(5):
            for c in range(2):
                if k < 4:
                    p, r = _pack(v[k][c], v[4 + k][c]), _pack(t2[k][c], t3[k][c])
                else:
                    p, r = _pack(t4[0][c], t4[1][c]), _pack(t4[2][c], t4[3][c])
                r4 = pltpu.roll(r, 4, 0)
                quads[0][c].append(jnp.where(low, p, r4))
                quads[1][c].append(jnp.where(low, r4, p))
                pin(quads[0][c][-1], 10)
            if k in late:
                pin(late[k], 8)
        held["lhs", b, gi] = [jnp.concatenate([jnp.concatenate(quads[q][c], 0) for c in range(2)], 1) for q in range(2)]
        held["s", b, gi] = special
        if g == 1:
            for s in range(3):
                xsp[s, pl.ds(8 * un, 8), :] = _pack(held["s", b, gi - 1][s], special[s])

    def kgen(b, gi):
        un, g = divmod(gi, 2)
        merged = []
        for q in range(2):
            rhs = jnp.concatenate([
                jnp.concatenate([jbuf[gi, c, pl.ds(32 * jj + 16 * q, 16), :] for jj in range(4)], 0)
                for c in range(2)], 1)
            lhs = held["lhs", b, gi][q]
            res = _dot(_bf(pinned(lhs) if CFG["pink"] else lhs), _bf(rhs), NT)
            vr = lambda i, h: res[16 * i + 8 * (h ^ q):16 * i + 8 * (h ^ q) + 8]
            rot = lambda t, k: pltpu.roll(t, 8 * k, 1, stride=4, stride_axis=0)
            ms = []
            for h in range(2):
                r = [rot(vr(k, h), k) for k in range(4)]
                ms.append(jnp.where(bit1, jnp.where(bit0, r[3], r[2]), jnp.where(bit0, r[1], r[0])))
            t = jnp.where(bit1, rot(vr(4, 1), 2), rot(vr(4, 0), 0))
            ms.append(jnp.where(odd != 0, pltpu.roll(t, 4, 1), t))
            merged.append(ms)
        if g == 0:
            held["m"] = merged
            return
        for q in range(2):
            for i in range(3):
                wd = _pack(held["m"][q][i], merged[q][i])
                kd[i, pl.ds(16 * un + 8 * q, 8), :] = wd
                if un < 7 and CFG["pinkd"]:
                    held.setdefault("late", []).append(wd)

    def ktile(b, t):
        ld = lambda i, h: jnp.concatenate([kd[i, pl.ds(16 * un + h, 8, stride=2), :] for un in range(8)], 0)
        if t < 4:
            return _bf(ld(t >> 1, t & 1))
        m = jnp.concatenate([bit0e] * 8, 0)
        return _bf(jnp.where(m, ld(2, 1), ld(2, 0)))

    def phi_table(s):
        for p in range(4):
            row = jnp.broadcast_to(phi[s:s + 1, 128 * p:128 * p + 128], (8, 128))
            words = _w(_bf(jnp.concatenate([_pack(row, row)] * 8, 0)).T)
            phit[s, pl.ds(64 * p, 64), :] = words
            held.setdefault("phi", []).append(words[56:])

    def specials(b):
        rhs = jnp.concatenate([xsp[min(s, 2), ds(0, 64, s), :] for s in range(4)], 0)
        sp = _dot(jnp.ones((16, 128), BF16), _bf(rhs), NT)[0:8]
        held["sp"] = (sp[:, :128], sp[:, 128:256], jnp.where(low, sp[:, 256:384], sp[:, 384:]))

    def khat(b, m):
        idx0 = sum(len(_TILES[i]) for i in range(m))
        acc = None
        for i, t in enumerate(_TILES[m]):
            tl = ktile(b, t)
            lhs = pinned4([wm[ds(256 * (idx0 + i) + 64 * p, 64, b), :] for p in range(4)])
            res = [_dot(lhs[p], tl, NT) for p in range(4)]
            acc = res if acc is None else [x + y for x, y in zip(acc, res)]
        for p in range(4):
            v = acc[p]
            if m in _FIX:
                s = list(_FIX).index(m)
                sp = jnp.concatenate([jnp.where(always, held["sp"][s], v[0:8])] * 16, 0)
                v = v + _bf(phit[s, ds(64 * p, 64, b), :]).astype(F32) * sp
            if m == 0 and p < 2:
                v = v + dsk[...].astype(F32)[b:b + 1, :]
            kh[m, pl.ds(128 * p, 128), :] = v
            acc[p] = v
            if CFG["gauss"] and p >= 2:
                kh[m, pl.ds(128 * (p + 2), 128), :] = v + acc[p - 2]

    def uhat(b, c):
        ev, od = [], []
        for k in range(8):
            wu = us[b, pl.ds(128 * c + 64 + 8 * k, 8), :]
            wl = perm8(us[b, pl.ds(128 * c + 56 - 8 * k, 8), :], rev8)
            u0, u1, l0, l1 = _unpack(wu, 0), _unpack(wu, 1), _unpack(wl, 0), _unpack(wl, 1)
            ev.append(_pack(u0 + l1, u1 + l0))
            od.append(_pack(u0 - l1, u1 - l0))
        lhs = pinned4([fwd[ds(64 * p, 64, c), :] for p in range(4)])
        res = [_dot(lhs[p], _bf(jnp.concatenate(ev if p < 2 else od, 0))) for p in range(4)]
        if CFG["gauss"]:
            res += [res[0] + res[2], res[1] + res[3]]
        for p, v in enumerate(res):
            uh[c, pl.ds(128 * p, 128), :] = v

    def conv_rows(r):
        row = 8 * r
        prev = None
        cost = [0, 0, 0]
        ld = lambda ref, j, o: ref[j, ds(o + row, 8, 0), :]
        for c in range(NC):
            if CFG["gauss"]:
                cur = [None] * 3
                for j in range(c + 1):
                    for comp in range(3):
                        t = ld(kh, j, CH * comp) * ld(uh, c - j, CH * comp)
                        cur[comp] = t if j == 0 else cur[comp] + t
                        cost[comp] += 2
                        if cost[comp] >= 4 * CFG["pstep"] and c - j >= 1:
                            pin(cur[comp], cost[comp])
                            cost[comp] = 0
                cur = (cur[0] - cur[1], cur[2] - cur[0] - cur[1])
                cost[0] += cost[1] + 1
                cost[1] = cost[2] + 2
                cost[2] = 0
            else:
                cur = [None, None]
                for j in range(c + 1):
                    kr, ki, ur, ui = ld(kh, j, 0), ld(kh, j, CH), ld(uh, c - j, 0), ld(uh, c - j, CH)
                    t = (kr * ur - ki * ui, kr * ui + ki * ur)
                    for comp in range(2):
                        cur[comp] = t[comp] if j == 0 else cur[comp] + t[comp]
                        cost[comp] += 4
                        if cost[comp] >= 4 * CFG["pstep"] and c - j >= 1:
                            pin(cur[comp], cost[comp])
                            cost[comp] = 0
            if prev is None:
                z = cur
            elif row < 128:
                z = (cur[0] - prev[1], cur[1] + prev[0])
            else:
                z = (cur[0] + prev[1], cur[1] - prev[0])
            prev = cur
            zz[c, pl.ds(row, 8), :] = z[0].astype(BF16)
            zz[c, pl.ds(CH + row, 8), :] = z[1].astype(BF16)
            if c >= 1:
                for comp in range(2):
                    pin(z[comp], cost[comp] + 2)
                    cost[comp] = 0

    todo = []
    clock = [0]

    def out_dma(src, dst):
        todo.append((clock[0] + 2, src, dst))

    def flush(force=False):
        while todo and (force or todo[0][0] <= clock[0]):
            _, src, dst = todo.pop(0)
            dma("out", src, dst)

    def inverse(b, c):
        lhs = pinned4([inv[ds(64 * i, 64, c), :] for i in range(4)])
        res = [_dot(lhs[i], _bf(hu(zz)[c, ds(64 * i, 64, b), :])) for i in range(4)]
        av, bv = res[0] + res[1], res[2] + res[3]
        up, dn = av + bv, av - bv
        for k in range(8):
            e, o = slice(16 * k, 16 * k + 8), slice(16 * k + 8, 16 * k + 16)
            ob[b, pl.ds(128 * c + 64 + 8 * k, 8), :] = _pack(up[e], up[o])
            ob[b, pl.ds(128 * c + 56 - 8 * k, 8), :] = perm8(_pack(dn[o], dn[e]), rev8)
        if b < 3:
            if c == NC - 1:
                out_dma(ob.at[b], hu(out_h).at[:, pl.ds(D + 128 * b, 128)])
        elif c % 2 == 1:
            rows = pl.ds(128 * (c - 1), 256)
            out_dma(ob.at[b, rows, :], hu(out_h).at[rows, pl.ds(D + 128 * b, 128)])

    st = {}

    def k_unit(t, b, i):
        tok = 512 * t + 128 * i
        pk = _phi(_dot(_bf(pinned(xrows(tok, 128, b))), _bf(pinned_rhs(wk[b, ds(0, 256, 4 * t + i), :]))))
        s = pk.reshape(16, 8, 128).sum(0)
        st["z", b] = st["z", b] + s if ("z", b) in st else s
        (pk0, pk1)[(4 * t + b) % 2][i] = _w(pk.astype(BF16).T)

    def g_unit(t, b, j):
        lhs = jnp.concatenate([(pk0, pk1)[(4 * t + b) % 2][i, ds(0, 64, j), :] for i in range(4)], 1)
        g = _dot(_bf(pinned(lhs)), _bf(pinned_rhs(xs[j, ds(256 * t, 256, 4 + b), :])))
        gt = (gt0, gt1, gt2, gt3)[b]
        gt[j] = g if t == 0 else gt[j, ds(0, 128, t), :] + g

    def put_heads(ref, idx, words):
        for hl in range(8):
            ref[(*idx, pl.ds(9 * hl, 8), slice(None))] = words[8 * hl:8 * hl + 8]

    def get_heads(ref, idx, tag):
        return jnp.concatenate([ref[(*idx, pl.ds(zoff[tag % NZ] + dp, 8, stride=9), slice(None))] for dp in range(8)], 0)

    def mid_w(b):
        for i in range(4):
            put_heads(wqt, (b, i), _w(_bf(wq[b, pl.ds(64 * i, 64), :]).T))

    def mid_z(b):
        z = jnp.broadcast_to(st["z", b].sum(0, keepdims=True), (8, 128))
        put_heads(zt, (b,), _w(_bf(jnp.concatenate([_pack(z, z)] * 8, 0)).T))
        v = _bf(get_heads(zt, (b,), 0)).astype(F32)
        zb[pl.ds(128 * b, 128), :] = v
        late.append(_w(v[120:]))

    def mid_kv(b):
        r128 = lax.broadcasted_iota(I32, (128, 128), 0)
        c128 = lax.broadcasted_iota(I32, (128, 128), 1)
        g = jnp.concatenate([(gt0, gt1, gt2, gt3)[b][j, ds(0, 128, 0), :] for j in range(4)], 1).astype(BF16)
        kv = _dot(g, _bf(wv[b]))
        st["kv", b] = jnp.where((r128 >> 4) == (c128 >> 4), kv, 0.0).astype(BF16)

    def mid_m(b):
        wob = jnp.concatenate([wo[j, pl.ds(64 * b, 64), :] for j in range(4)], 1)
        m = _dot(st["kv", b], _bf(wob))
        for j in range(4):
            put_heads(mm, (j, b), _w(m[:, 128 * j:128 * j + 128].astype(BF16)))

    def q_unit(t, b):
        lhs = jnp.concatenate([get_heads(wqt, (b, i), t) for i in range(4)], 1)
        pq = _phi(_dot(_bf(pinned(lhs)), _bf(xrows(128 * t, 128, 8 + b)), NT))
        blk = [pq[8 * v:8 * v + 8] for v in range(16)]
        rd = []
        for g in range(2):
            s = _sum([blk[v] * zb[ds(128 * b + 8 * v, 8, t), :] for v in range(g, 16, 2)])
            den = s + perm8(s, sub ^ 1) + 1e-6
            r = pltpu.reciprocal(den, approx=True)
            rd.append(r * (2.0 - den * r))
        (pq0, pq1, pq2)[t % 3][b] = _w(jnp.concatenate([blk[v] * rd[v % 2] for v in range(16)], 0).astype(BF16).T)

    def o_unit(t, j):
        lhs = jnp.concatenate([(pq0, pq1, pq2)[t % 3][b, ds(0, 64, j), :] for b in range(4)], 1)
        rhs = jnp.concatenate([get_heads(mm, (j, b), t) for b in range(4)], 0)
        oa[j, pl.ds(128 * t, 128), :] = _dot(_bf(pinned(lhs)), _bf(pinned_rhs(rhs))).astype(BF16)
        if j == 3 and (t % 2 == 1 or t == 14):
            t0 = t - 1 if (t % 2 == 1 and t != 15) else t
            rows = pl.ds(128 * t0, 128 * (t + 1 - t0))
            for jj in range(4):
                out_dma(oa.at[jj, rows, :], out_h.at[rows, pl.ds(128 * jj, 128)])

    au = []
    P = functools.partial
    macro = [(t, b) for t in range(4) for b in range(4)]
    order = ((0, 0), (0, 1), (1, 0), (0, 2), (1, 1), (0, 3), (1, 2), (1, 3))
    for n in range(len(macro) + 1):
        for kind, i in {7: sorted(order), 8: sorted(order, reverse=True, key=lambda e: e[0]),
                        9: sorted(order)}.get(n, order):
            if kind == 0 and n < len(macro):
                t, b = macro[n]
                au.append((P(k_unit, t, b, i), [("x", i), ("wk", b)] if t == 0 else [], "k"))
            if kind == 1 and n > 0:
                au.append((P(g_unit, *macro[n - 1], i), [], "g"))
        if n in (14, 15):
            au.append((P(mid_kv, n - 14), [], "n"))
    mid = [(q_unit, 0, 0), (q_unit, 0, 1), (mid_kv, 2), (q_unit, 0, 2), (mid_kv, 3), (q_unit, 0, 3),
           (mid_m, 0), (mid_m, 1), (q_unit, 1, 0), (mid_m, 2), (q_unit, 1, 1), (q_unit, 1, 2), (mid_m, 3),
           (q_unit, 1, 3)]
    au += [(P(*e), [], "q" if e[0] is q_unit else "n") for e in mid]
    for t in range(16):
        for kind, i in order:
            if kind == 0 and t + 2 < 16:
                au.append((P(q_unit, t + 2, i), [], "q"))
            if kind == 1:
                au.append((P(o_unit, t, i), [], "o"))
    n_a = len(au)
    side = {90: [P(mid_w, 0)], 94: [P(mid_w, 1)], 98: [P(mid_w, 2)], 102: [P(mid_w, 3)],
            106: [P(mid_z, 0)], 114: [P(mid_z, 1)], 122: [P(mid_z, 2)], 126: [P(mid_z, 3)]}

    def run_a(n):
        while au and n > 0:
            idx = n_a - len(au)
            unit = au.pop(0)
            begin(unit[2])
            unit[0]()
            for f in side.get(idx, []):
                f()
            clock[0] += 1
            n -= unit[2] != "n"

    def quiet(units):
        flush()
        for _, needs, _ in au[:units]:
            wait(*[n for n in needs if n in batches])

    gq = []
    tails = []

    def gen_next(n):
        for _ in range(n):
            if gq:
                b, gi = gq.pop(0)
                k = len(pins)
                gen_vpu(b, gi)
                if CFG["split"]:
                    mine = pins[k:]
                    del pins[k:]
                    cut = (len(mine) * CFG["split"]) // 100
                    head, old = mine[:cut], tails[:]
                    tails[:] = mine[cut:]
                    keyed = [((i + 0.5) / len(head), p) for i, p in enumerate(head)]
                    keyed += [((i + 0.25) / len(old), p) for i, p in enumerate(old)]
                    pins.extend(p for _, p in sorted(keyed, key=lambda e: e[0]))
            elif tails:
                pins.extend(tails)
                tails.clear()

    def gen_phase(b, gen_a):
        done = 0
        ulast = CFG["u0"] if b == 0 else 0
        uslots = [ulast + ((16 - ulast) * (2 * c + 1)) // 16 for c in range(NC)]
        for gi in range(16):
            want = (gen_a * (gi + 1) + 8) // 16
            quiet(want - done)
            while gq and gq[0] <= (b, gi + CFG["look"]):
                gen_next(1)
            if gi + CFG["look"] == 16 and tails:
                pins.extend(tails)
                tails.clear()
            nb = (1 if (gi % 2 == 0 and b > 0) else 0) + uslots.count(gi)
            if gi % 2 == 1:
                late.extend(held.pop("late", []))
            drain_over(want - done, nb + 0.6 * CFG["pink"])
            run_a(want - done)
            done = want
            if gi % 2 == 0 and b > 0:
                begin("b")
                inverse(b - 1, gi // 2)
                clock[0] += 1
            for c in range(NC):
                if uslots[c] == gi:
                    if b == 0:
                        wait(("wk", 2))
                    begin("b")
                    uhat(b, c)
                    clock[0] += 1
            begin("b")
            kgen(b, gi)

    def khat_phase(b):
        ahead = CFG["ahead"] if b < 3 else 0
        quiet(CFG["kh_a"])
        for i in range(CFG["kh_a"]):
            run_a(1)
            if i == 1:
                specials(b)
        for m in range(NC):
            if b == 0 and m == 0:
                wait("wm")
            if b > 0 and m % 2 == 0 and m // 2 < ahead:
                gen_next(1)
                drain_over(0, 2)
            khat(b, m)

    def conv_phase(conv_a, b):
        quiet(1)
        if b < 2 and not CFG["tb"]:
            wait(("c0", "rest")[b])
        run_a(1)
        done = 1
        extra = 0
        if b < 3:
            extra = max(0, CFG["look"] + (CFG["ahead"] if b == 0 else 0) - (16 - sum(1 for x in gq if x[0] == b + 1)))
        slots = 32 + extra * 1.4
        for r in range(32 + extra):
            pos = r + 1 if r < 32 else 32 + (r - 31) * 1.4
            want = 1 + int(np.ceil((conv_a - 1) * pos / slots - 1e-9))
            quiet(want - done)
            if r < 32:
                conv_rows(r)
            else:
                gen_next(1)
            if want > done:
                drain_over(want - done)
                run_a(want - done)
                done = want

    if CFG["tb"]:
        wait(*batches)
        for b in range(4):
            st["z", b] = jnp.zeros((8, 128), F32)
        del au[:CFG["skip"]]
        if CFG["tb"] == 1:
            conv_phase(47, 3)
            inverse(3, 7)
        elif CFG["tb"] == 2:
            gq += [(1, gi) for gi in range(16)]
            gen_phase(1, CFG["gen_a"])
            run_a(2)
            specials(1)
            run_a(1)
            khat(1, 3)
            ob[0, pl.ds(0, 64), :] = _w(kh[3, ds(0, 64, 0), :] + uh[2, ds(0, 64, 0), :])
        ob[1, pl.ds(0, 64), :] = _w(gt0[0, ds(0, 64, 0), :] + gt1[0, ds(0, 64, 0), :] + gt2[0, ds(0, 64, 0), :] + gt3[0, ds(0, 64, 0), :])
        out_dma(ob.at[0], hu(out_h).at[:, pl.ds(0, 128)])
        out_dma(ob.at[1], hu(out_h).at[:, pl.ds(128, 128)])
        out_dma(oa.at[1], out_h.at[:, pl.ds(256, 128)])
    else:
        gq += [(b, gi) for b in range(4) for gi in range(16)]
        ends = [CFG["e0"], CFG["e1"], CFG["e2"], 256 - CFG["tail"]]
        used = 0
        for i in range(3):
            phi_table(i)
        quiet(1)
        gen_next(1)
        drain_over(CFG["pre"])
        for _ in range(CFG["pre"]):
            quiet(1)
            run_a(1)
        for b in range(4):
            quota = ends[b] - used
            late.extend(held.pop("phi", []))
            used = ends[b]
            gen_a = (CFG["gen_a0"], CFG["gen_a"], CFG["gen_a2"], CFG["gen_a2"])[b]
            if b == 1:
                wait("g1")
            gen_phase(b, gen_a)
            khat_phase(b)
            conv_phase(quota - gen_a - CFG["kh_a"] - (CFG["pre"] if b == 0 else 0), b)
        for c in range(NC):
            run_a(1)
            inverse(3, c)
            clock[0] += 1
            flush()
        while au:
            run_a(1)
            flush()
    flush(True)
    wait(*batches)


@jax.jit
def pallas_concat_heads__linear_attn_block__ssm_conv_s4__prompt_kernel(A_x, A_wqkv, A_wo, B_u, B_A_re, B_A_im, B_B_re, B_B_im, B_C_re, B_C_im, B_log_dt, B_Dskip):
    consts = _constants()
    ins = (A_x.reshape(L, D), A_wqkv, A_wo, B_u.reshape(L, D), B_A_re, B_A_im, B_B_re, B_B_im,
           B_C_re, B_C_im, B_log_dt.reshape(4, 128), B_Dskip.reshape(4, 128)) + consts
    vm = pltpu.VMEM
    scratch = [
        vm((4, L // 2, 128), U32), *[vm((4, D // 2, 128), U32)] * 4,
        vm((4, L // 2, 128), U32), vm((6, D // 2, N), U32), pltpu.SMEM((2, 128), U32), vm((4, 128), BF16),
        vm((256, 128), U32), vm((256, 128), U32), vm((9 * 256, 128), U32), vm((8, 512), F32),
        vm((4, 4, 72, 128), U32), *[vm((4, 128, 128), F32)] * 4, vm((4, 4, 72, 128), U32), vm((D, 128), F32), vm((4, 72, 128), U32),
        vm((16, 2, 128, 128), U32), vm((3, 128, 128), U32), vm((3, 64, 128), U32),
        vm((NC, 768, 128), F32), vm((NC, 768, 128), F32), vm((NC, 512, 128), BF16),
        vm((4, L // 2, 128), U32), vm((4, L, 128), BF16),
        *[vm((4, 64, 128), U32)] * 5, vm((3, 256, 128), U32), pltpu.SMEM((2 * NZ,), I32),
        pltpu.SemaphoreType.DMA((12,)),
    ]
    out = pl.pallas_call(
        _kernel,
        out_shape=jax.ShapeDtypeStruct((L, 2 * D), BF16),
        in_specs=[pl.BlockSpec(memory_space=pl.ANY)] * len(ins),
        out_specs=pl.BlockSpec(memory_space=pl.ANY),
        scratch_shapes=scratch,
        compiler_params=pltpu.CompilerParams(vmem_limit_bytes=100 * 2 ** 20,
                                              flags={"XLA_TPU_RESCHEDULE_DMA_DONES": True}),
        name="fused_k",
    )(*ins)
    return out.reshape(1, L, 2 * D)
```

```python
import functools

import jax
import jax.numpy as jnp
import ml_dtypes
import numpy as np
from jax import lax
import jax.experimental.pallas as pl
import jax.experimental.pallas.tpu as pltpu

F32, BF16, U32, I32 = jnp.float32, jnp.bfloat16, jnp.uint32, jnp.int32

L = 2048
D = 512
N = 128
CH = 256
NC = L // CH
NZ = 16
NN = (((1,), (0,)), ((), ()))
NT = (((1,), (1,)), ((), ()))

_OFFSETS = ((0, 2, 4, 6), (1, 3, 5, 7), (256, 258, 260, 262), (512, 516, 768, 772), (1024, 1280, 1536, 1792))
_POWERS = (0, 1, 2, 4, 8, 16, 3, 6, 12, 24, 5, 10, 7, 14, 20, 28, 9, 18, 11, 22, 13, 26, 15, 30,
           17, 19, 21, 23, 25, 27, 29, 31)
_TILES = ((0, 1), (2,), (3,), (3,), (4,), (4,), (4,), (4,))
_ZERO = 24
_SPARE = 32
_SLOTS = (((0, 0), (0, 1), (5, 0), (6, 0)), ((1, 0), (2, 0), (5, 1), (6, 1)), ((3, 0), (4, 0), (7, 0), (7, 1)),
          ((1, 1), (2, 1), (3, 1), (4, 1)), ((0, 2), (0, 3), (5, 2), (6, 2)), ((1, 2), (2, 2), (3, 2), (4, 2)),
          ((7, 2), (7, 3), (5, 3), (6, 3)), ((1, 3), (2, 3), (3, 3), (4, 3)))
_K_IM, _K_ROWS = 72, 144
_U_IM, _U_ROWS = 264, 528
_SEMS = 4

_LOAD = dict(p=(16, 180), k=(16, 32, 32, 136, 168, 216, 192), q=(16, 32, 32, 200, 216, 272, 224),
             o=(16, 32, 32, 40, 40, 56, 40), g=(48, 64), kv=(150, 170), m=(64, 230), z=(60,),
             kgen=(30, 34), uhat=(80,), inv=(75,), khat=(35, 75), tiles=(40,))


@functools.cache
def _constants():
    bf = ml_dtypes.bfloat16
    lag = np.arange(L).astype(np.float32).astype(bf).astype(np.int64)
    f = np.concatenate([v for q in range(4) for v in (np.arange(q, 128, 4), 255 - np.arange(q, 128, 4))])
    om = 2 * np.pi * (f + 0.5) / (2 * CH)
    s = np.arange(128) + 0.5
    fwd = np.concatenate([np.cos(om[:, None] * s), -np.sin(om[:, None] * s)], 0)
    low = om.reshape(4, 2, 32)[:, 0].reshape(-1)
    t = np.arange(0, 128, 2)
    inv = np.concatenate([np.cos(low * np.concatenate([t, [128], np.zeros(15)])[:, None]),
                          np.cos(low * (t + 1)[:, None]),
                          np.sin(low * np.where(t, t, 128)[:, None]),
                          np.sin(low * (t + 1)[:, None])], 0) / CH

    def lanes(tile):
        shift = 4 * (tile & 1 if tile < 4 else 0)
        out = np.zeros(128, np.int64)
        for i in range(4):
            for j in range(32):
                out[(32 * (j >> 3) + (j & 7) + 24 + 8 * i + shift) % 128] = _OFFSETS[tile][i] + 8 * _POWERS[j]
        return out

    def spectrum(m, lags):
        phase = np.exp(-1j * om[:, None] * (np.arange(CH)[None, :] - 0.5))
        taps = lambda c: phase @ (lag[CH * c:CH * (c + 1), None] == lags[None, :]).astype(np.float64)
        w = taps(m)
        if m >= 5 or m == 2:
            w = w + 1j * np.where(f % 2, -1, 1)[:, None] * taps(m - 1)
        return np.stack([w.real.reshape(4, 64, -1), w.imag.reshape(4, 64, -1)], 1).reshape(4, 128, 128)

    assert lanes(0)[_ZERO] == 0 and lanes(4)[_ZERO] == 4 * CH and lanes(3)[28] == 2 * CH
    maps = [(m, lanes(tile)) for m in range(NC) for tile in _TILES[m]]
    for m, lags in maps:
        if m in (3, 7):
            assert lags[_SPARE] < CH * m
            lags[_SPARE] = CH * (m + 1)
    mats = [spectrum(m, lags) for m, lags in maps]
    first = lambda q: mats[q % 2].reshape(2, 2, 2, 2, 32, 128)[q // 2, :, :, 0].reshape(128, 128)
    taps = np.concatenate([mats[m + 1][q] if m else first(q) for slots in _SLOTS for m, q in slots], 0)
    return fwd.astype(bf), inv.astype(bf), taps.astype(bf), np.zeros((128,), np.int32)


def _bf(v):
    return pltpu.bitcast(v, BF16)


def _w(v):
    return pltpu.bitcast(v, U32)


def _pack(a, b):
    return pltpu.pack_elementwise([a, b], packed_dtype=BF16)


def _unpack(v, i):
    return pltpu.unpack_elementwise(v, index=i, packed_dtype=BF16, unpacked_dtype=F32)


def _dot(a, b, dims=NN):
    return lax.dot_general(a, b, dims, preferred_element_type=F32)


def _cmul(a, b):
    return a[0] * b[0] - a[1] * b[1], a[0] * b[1] + a[1] * b[0]


def _csq(a):
    t = a[0] * a[1]
    return a[0] * a[0] - a[1] * a[1], t + t


def _phi(t):
    return jnp.where(t > 0, t + 1.0, jnp.exp(t)) + 1e-6


def _sum(xs):
    return functools.reduce(lambda a, b: a + b, xs)


def _kernel(x_h, wqkv_h, wo_h, u_h, are_h, aim_h, bre_h, bim_h, cre_h, cim_h, ldt_h, dsk_h,
            fwd_h, inv_h, taps_h, zero_h, out_h,
            dsk, xs, wq, wk, wv, wo, us, par, ldt, fwd, inv, wm,
            wqt, gt0, gt1, mm, zb, zt, jbuf, kd, uh, ob, oa,
            pk0, pk1, kvt, kedge, kx, k0, dcol, zs, sems, *more):
    pqs, wkc, xc, kh, klast, zz = more[:8], more[8:10], more[10:18], more[18:22], more[22:24], more[24:]
    P = functools.partial
    hu = lambda r: r.bitcast(U32)
    held = {}

    planned, batches, free = {}, {}, list(range(_SEMS))
    late_batches = ("w2", "x6", "second", "rest")

    def dma(batch, src, dst):
        planned.setdefault(batch, []).append((src, dst))

    def start():
        while planned and free:
            batch, sem = next(iter(planned)), free.pop(0)
            batches[batch] = sem, [pltpu.make_async_copy(src, dst, sems.at[sem]) for src, dst in planned.pop(batch)]
            for c in batches[batch][1]:
                c.start()

    def wait(*names):
        for n in names:
            assert n not in planned
            if n in batches:
                if n in late_batches:
                    dsk[pl.ds(32 + 8 * late_batches.index(n), 8), :] = _w(held["last"])
                sem, copies = batches.pop(n)
                for c in copies:
                    c.wait()
                free.append(sem)
                start()

    def x_dma(batch, r0, n):
        rows = pl.ds(r0 // 2, n // 2)
        for j in range(4):
            dma(batch, hu(x_h).at[rows, pl.ds(128 * j, 128)], xs.at[j, rows, :])

    def col_dma(batch, src, c0, dst):
        dma(batch, hu(src).at[:, pl.ds(c0, 128)], dst)

    def par_dma(batch, r0, r1):
        for i, r in enumerate((are_h, aim_h, bre_h, bim_h, cre_h, cim_h)):
            dma(batch, hu(r).at[pl.ds(r0, r1 - r0), :], par.at[i, pl.ds(r0, r1 - r0), :])

    def taps_dma(batch, u0, u1):
        rows = pl.ds(256 * u0, 256 * (u1 - u0))
        dma(batch, hu(taps_h).at[rows, :], wm.at[rows, :])

    dma("first", zero_h, zs)
    dma("first", hu(ldt_h), ldt)
    par_dma("first", 0, 16)
    col_dma("first", wqkv_h, D, wk.at[0])
    x_dma("first", 0, 128)
    x_dma(("x", 1), 128, 128)
    col_dma(("wk", 1), wqkv_h, D + 128, wk.at[1])
    par_dma(("wk", 2), 16, 64)
    col_dma(("wk", 2), wqkv_h, D + 256, wk.at[2])
    col_dma(("wk", 3), wqkv_h, D + 384, wk.at[3])
    x_dma(("x", 2), 256, 128)
    x_dma(("x", 3), 384, 128)
    x_dma(("x", 4), 512, 256)
    x_dma(("x", 6), 768, 256)
    dma("u0", hu(fwd_h), fwd)
    dma("u0", hu(dsk_h), dsk.at[pl.ds(0, 2), :])
    for i in range(2):
        dma(("u0", "u1")[i], hu(u_h).at[pl.ds(512 * i, 512), pl.ds(0, 128)], us.at[0, pl.ds(512 * i, 512), :])
    par_dma("u1", 64, 128)
    x_dma("x4", 1024, 512)
    taps_dma("w0", 0, 3)
    taps_dma("w1", 3, 4)
    taps_dma("w2", 4, 6)
    x_dma("x6", 1536, 512)
    taps_dma("x6", 6, 8)
    dma("second", hu(inv_h), inv.at[pl.ds(0, 136), :])
    col_dma("second", u_h, 128, us.at[1])
    par_dma("second", 128, 256)
    for b in range(4):
        col_dma("second", wqkv_h, 128 * b, wq.at[b])
    for b in range(2, 4):
        col_dma("rest", u_h, 128 * b, us.at[b])
    for b in range(4):
        col_dma("rest", wqkv_h, 2 * D + 128 * b, wv.at[b])
    for b in range(4):
        col_dma("rest", wo_h, 128 * b, wo.at[b])
    start()
    wait("first")

    clock = [0, 0]
    todo, sent = [], []

    def send(src, dst):
        todo.append((clock[0] + 2, src, dst))

    def flush(everything=False):
        while todo and (everything or todo[0][0] <= clock[0]):
            assert not planned and free
            _, src, dst = todo.pop(0)
            sent.append(pltpu.make_async_copy(src, dst, sems.at[free[0]]))
            sent[-1].start()

    zoff = [zs[i] for i in range(NZ)]

    def ds(first, size, tag):
        return pl.ds(pl.multiple_of(zoff[tag % NZ] + first, 8), size)

    sub = lax.broadcasted_iota(I32, (8, 128), 0)
    lane = lax.broadcasted_iota(I32, (8, 128), 1)
    odd = sub & 1
    block = (lane + (104 - 4 * odd)) >> 3
    bit0 = (block & 1) != 0
    bit1 = (block & 2) != 0
    bit0e = (((lane + 104) >> 3) & 1) != 0
    low = sub < 4
    rev8 = 7 - sub
    rev4 = sub ^ 3
    always = [(lane * sub) >= -n for n in range(3)]
    perm8 = lambda v, idx: jnp.take_along_axis(v, idx, axis=0)

    pins = []
    timed = []
    late = []
    share = []
    credit = [0.0, 0]

    def pin(v, cost):
        n = len(pins)
        while n and pins[n - 1][2] > credit[1]:
            n -= 1
        pins.insert(n, (_w(v), cost, credit[1]))

    def settle(words, rows):
        timed.append((clock[1] + rows, _w(words[-8:])))
        timed.sort(key=lambda e: e[0])
        return words

    def pinned(words):
        rows = []
        cols = words.shape[1] // 128
        for i in range(words.shape[0] // 8):
            row = []
            for j in range(cols):
                v = words[8 * i:8 * i + 8, 128 * j:128 * j + 128]
                credit[0] += share[i] / cols
                ties = []
                if timed and timed[0][0] <= clock[1] + i:
                    ties.append(timed.pop(0)[1])
                while pins and credit[0] >= 0.5 * pins[0][1] and len(ties) < (3 if clock[0] < 3 else 1):
                    ties.append(pins[0][0])
                    credit[0] -= pins.pop(0)[1]
                for n, tie in enumerate(ties):
                    v = jnp.where(always[n], v, tie)
                row.append(v)
            rows.append(jnp.concatenate(row, 1))
        if not pins:
            credit[0] = min(credit[0], 0.0)
        return jnp.concatenate(rows, 0)

    def pinned4(tiles):
        v = pinned(jnp.concatenate(tiles, 1))
        return [_bf(v[:, 128 * p:128 * p + 128]) for p in range(4)]

    def pinned_rhs(words):
        if not late:
            return words
        v = [words[8 * i:8 * i + 8] for i in range(words.shape[0] // 8)]
        for j in range(words.shape[0] // 64):
            if late:
                v[8 * j + 7] = jnp.where(always[0], v[8 * j + 7], late.pop(0))
        return jnp.concatenate(v, 0)

    def factors(b, gi):
        un, g = divmod(gi, 2)
        rows = pl.ds(64 * b + 8 * un, 8)
        are, aim, bre, bim, cre, cim = [_unpack(par[i, rows, :], g) for i in range(6)]
        dt = [jnp.full((8, 128), ldt[b // 2, 16 * un + 2 * i + g], U32) for i in range(8)]
        for m in (odd != 0, (sub & 2) != 0, sub >= 4):
            dt = [jnp.where(m, dt[i + 1], dt[i]) for i in range(0, len(dt), 2)]
        pin(dt[0], 15)
        dt = jnp.exp(_unpack(dt[0], b % 2)).astype(BF16).astype(F32)
        pin(dt, 10)
        t = (dt * aim) * np.float32(1.0 / (2.0 * np.pi))
        magic = np.float32(1.5 * 2.0 ** 23)
        x = (t - ((t + magic) - magic)) * np.float32(np.pi / 2.0)
        z = x * x
        pin(z, 9)
        sn = x + x * z * (np.float32(-1.6666654611e-1)
                          + z * (np.float32(8.3321608736e-3) + z * np.float32(-1.9515295891e-4)))
        cs = 1.0 + z * (np.float32(-0.5) + z * (np.float32(4.166664568298827e-2) + z * (
            np.float32(-1.388731625493765e-3) + z * np.float32(2.443315711809948e-5))))
        r = jnp.exp((dt * are) * 0.25)
        a = (r * cs, r * sn)
        pin(cs, 12)
        pin(a[0], 8)
        pin(a[1], 8)
        for i in range(5):
            a = _csq(a)
            if i == 1:
                a1c = (a[0], -a[1])
            if i == 3:
                a4c = (a[0], -a[1])
            if i in (1, 4):
                pin(a[0], 12)
        a8 = (perm8(a[0], rev4), perm8(a[1], rev4))
        made = {0: (jnp.ones_like(dt), jnp.zeros_like(dt)), 1: a8}

        def power(j):
            if j not in made:
                made[j] = _cmul(power(j - 2), power(2)) if j % 2 else _csq(power(j // 2))
            return made[j]

        for k in range(16):
            dst = pl.ds(32 * (k >> 2) + (k & 3), 8, stride=4)
            for c in range(2):
                words = _pack(power(_POWERS[2 * k])[c], power(_POWERS[2 * k + 1])[c])
                jbuf[gi, c, dst, :] = words
            pin(words, 14)
        e = power(32)
        a256c = (perm8(e[0], rev4), -perm8(e[1], rev4))
        quads = [[[None] * 5, [None] * 5], [[None] * 5, [None] * 5]]
        pack = lambda lo, hi: [_pack(lo[c], hi[c]) for c in range(2)]

        def quad(k, p, r, cost):
            for c in range(2):
                r4 = pltpu.roll(r[c], 4, 0)
                quads[0][c][k] = jnp.where(low, p[c], r4)
                quads[1][c][k] = jnp.where(low, r4, p[c])
                pin(quads[0][c][k], cost)

        def times(v, a, anchor=True):
            v = _cmul(v, a)
            if anchor:
                pin(v[0], 9)
            return v

        cb = _cmul((cre, cim), (bre, bim))
        v0 = (cb[0] * dt, -(cb[1] * dt))
        pin(v0[0], 9)
        v4 = times(v0, a4c)
        v256 = times(v0, a256c, False)
        v512 = times(v256, a256c)
        v1 = times(v0, a1c)
        quad(0, pack(v0, v1), pack(v256, v512), 6)
        v260 = times(v4, a256c, False)
        v768 = times(v512, a256c)
        v5 = times(v4, a1c)
        quad(2, pack(v4, v5), pack(v260, v768), 6)
        v1024 = times(v768, a256c)
        v1280 = times(v1024, a256c)
        v1536 = times(v1280, a256c)
        v1792 = times(v1536, a256c, False)
        held["2048", b, gi] = v1792[0] * a256c[0] - v1792[1] * a256c[1]
        if g == 1:
            klast[b % 2][pl.ds(8 * un, 8), :] = _pack(held.pop(("2048", b, gi - 1)), held.pop(("2048", b, gi)))
        quad(4, pack(v1024, v1280), pack(v1536, v1792), 6)
        v516 = times(v260, a256c)
        v2, v6 = times(v1, a1c), times(v5, a1c)
        quad(1, pack(v2, times(v2, a1c, False)), pack(times(v2, a256c, False), v516), 9)
        quad(3, pack(v6, times(v6, a1c, False)), pack(times(v6, a256c, False), times(v516, a256c)), 9)
        held["rows", b, gi] = [jnp.concatenate([jnp.concatenate(quads[q][c], 0) for c in range(2)], 1) for q in range(2)]

    def kgen(b, gi):
        un, g = divmod(gi, 2)
        merged = []
        rows = pinned(jnp.concatenate(held.pop(("rows", b, gi)), 1))
        for q in range(2):
            rhs = jnp.concatenate([
                jnp.concatenate([jbuf[gi, c, pl.ds(32 * jj + 16 * q, 16), :] for jj in range(4)], 0)
                for c in range(2)], 1)
            res = _dot(_bf(rows[:, 256 * q:256 * q + 256]), _bf(rhs), NT)
            held["last"] = res[:8]
            part = lambda i, h: res[16 * i + 8 * (h ^ q):16 * i + 8 * (h ^ q) + 8]
            rot = lambda t, k: pltpu.roll(t, 8 * k, 1, stride=4, stride_axis=0)
            ms = []
            for h in range(2):
                r = [rot(part(k, h), k) for k in range(4)]
                ms.append(jnp.where(bit1, jnp.where(bit0, r[3], r[2]), jnp.where(bit0, r[1], r[0])))
            t = jnp.where(bit1, rot(part(4, 1), 2), rot(part(4, 0), 0))
            ms.append(jnp.where(odd != 0, pltpu.roll(t, 4, 1), t))
            merged.append(ms)
        if g == 0:
            held["taps"] = merged
            return
        for q in range(2):
            for i in range(3):
                kd[i, pl.ds(16 * un + 8 * q, 8), :] = _pack(held["taps"][q][i], merged[q][i])

    def ktile(tile, zero=0):
        load = lambda i, h: jnp.concatenate([kd[i, pl.ds(zero + 16 * un + h, 8, stride=2), :] for un in range(8)], 0)
        if tile < 4:
            return load(tile >> 1, tile & 1)
        return jnp.where(jnp.concatenate([bit0e] * 8, 0), load(2, 1), load(2, 0))

    def columns(row):
        return _w(_bf(jnp.concatenate([_pack(row, row)] * 8, 0)).T)

    def skip_table():
        for b in range(4):
            words = columns(_unpack(jnp.broadcast_to(dsk[pl.ds(b // 2, 1), :], (8, 128)), b % 2))
            dcol[b] = jnp.where(jnp.concatenate([lane == _ZERO] * 8, 0), words, 0)
            held.setdefault("skip", []).append(words[56:])

    def special_tiles(b):
        k0[...] = _pack(*[_unpack(ktile(0), h) + _unpack(dcol[b], h) for h in range(2)])
        spare = jnp.concatenate([lane == _SPARE] * 8, 0)
        rhs = jnp.concatenate([klast[b % 2][ds(0, 64, s), :] for s in range(4)], 0)
        sums = _dot(jnp.ones((16, 128), BF16), _bf(rhs), NT)[0:8]
        sums = [jnp.where(always[0], sums[:, 256 * h:256 * h + 128], sums[:, 256 * h + 128:256 * h + 256])
                for h in range(2)]
        for s, words in enumerate((pltpu.roll(ktile(4), _SPARE - _ZERO, 1), columns(jnp.where(always[1], *sums)))):
            words = jnp.where(spare, words, ktile(3 + s))
            kx[s] = words
            held["tile", (5 + s, 1)] = words[56:]
        row = _unpack(_w(_bf(ktile(3)).T)[8:16], 0)
        kedge[b] = settle(jnp.where(sub == 7, jnp.broadcast_to(row[6:7], (8, 128)), 0.0), 64)

    def khat(b, u):
        lhs = pinned4([wm[ds(256 * u + 64 * i, 64, b), :] for i in range(4)])

        def keep(m, q, re, im):
            if m < 5:
                pr, pi = held.pop(("k", q), (None, None))
                if m < 4:
                    held["k", q] = re, im
                if m > 0:
                    turn = [(re[h] - pi[h], im[h] + pr[h]) if (q + n) % 2 == 0 else (re[h] + pi[h], im[h] - pr[h])
                            for n, h in enumerate((slice(0, 32), slice(32, 64)))]
                    re, im = [jnp.concatenate([e[c] for e in turn], 0) for c in range(2)]
            kh[q][m, pl.ds(0, 64), :] = re
            kh[q][m, pl.ds(_K_IM, 64), :] = im

        for n, (m, q) in enumerate(_SLOTS[u]):
            if m in (3, 7):
                rhs = kx[m // 4, ds(0, 64, q), :]
            elif m == 0 and q % 2 == 0:
                rhs = k0[ds(0, 64, q), :]
            else:
                rhs = ktile(_TILES[m][-1], zoff[4 * (u % 4) + n])
            if ("tile", (m, q)) in held:
                late.append(held.pop(("tile", (m, q))))
                rhs = pinned_rhs(rhs)
            v = _dot(lhs[n], _bf(rhs), NT)
            held["last"] = v[:8]
            if m:
                keep(m, q, v[:64], v[64:])
            elif q % 2 == 0:
                even = v
            else:
                plus, minus = even + v, even - v
                for h in range(2):
                    re, im = slice(64 * h, 64 * h + 32), slice(64 * h + 32, 64 * h + 64)
                    keep(0, q - 1 + h, jnp.concatenate([plus[re], minus[im]], 0),
                         jnp.concatenate([plus[im], minus[re]], 0))

    def uhat(b, c):
        ev, od = [], []
        for k in range(8):
            up = us[b, pl.ds(128 * c + 64 + 8 * k, 8), :]
            down = perm8(us[b, pl.ds(128 * c + 56 - 8 * k, 8), :], rev8)
            u0, u1, d0, d1 = _unpack(up, 0), _unpack(up, 1), _unpack(down, 0), _unpack(down, 1)
            ev.append(_pack(u0 + d1, u1 + d0))
            od.append(_pack(u0 - d1, u1 - d0))
        lhs = pinned4([fwd[ds(64 * p, 64, c), :] for p in range(4)])
        rhs = pinned_rhs(jnp.concatenate(ev, 0)), pinned_rhs(jnp.concatenate(od, 0))
        res = [_dot(lhs[p], _bf(rhs[p // 2])) for p in range(4)]
        held["last"] = res[0][:8]
        for p, v in enumerate(res):
            uh[c, pl.ds(_U_IM * (p // 2) + 128 * (p % 2), 128), :] = v

    def convolve(r, c0):
        q = r // 2
        rest = [0]

        def product(row, whole):
            k = lambda j, o: kh[q][j, ds(_K_IM * o + row, 8, c0), :]
            u = lambda j, o: uh[j, ds(_U_IM * o + 64 * q + row, 8, c0), :]
            acc, cost = {}, {}
            for j in range(c0 + 2):
                for c in range(max(c0, j), c0 + 2):
                    t = _cmul((k(j, 0), k(j, 1)), (u(c - j, 0), u(c - j, 1)))
                    for o in range(2):
                        acc[c, o] = t[o] if j == 0 else acc[c, o] + t[o]
                        cost[c, o] = cost.get((c, o), 0) + (4 if j else 3)
                        if j % 2 and (j < c or whole):
                            pin(acc[c, o], cost.pop((c, o)))
            rest[0] += sum(cost.values())
            return acc

        z = []
        for h in range(2):
            x = product(16 * (r % 2) + 8 * h, True)
            y = product(16 * (r % 2) + 8 * h + 32, h == 0)
            z.append({c: (x[c, 0] + y[c, 0], x[c, 0] - y[c, 0], x[c, 1] - y[c, 1], x[c, 1] + y[c, 1])
                      for c in (c0, c0 + 1)})
        for c in (c0, c0 + 1):
            for i in range(4):
                words = _w(jnp.concatenate([z[0][c][i], z[1][c][i]], 0).astype(BF16))
                zz[c // 2][c % 2, pl.ds(64 * i + 8 * r, 8), :] = words
                pin(words, rest[0] / 8 + 3)

    def inverse(b, c):
        order = [(c + n) % 4 for n in range(4)]
        lhs = pinned(jnp.concatenate([inv[ds((0, 40, 72, 104)[i], 32, c), :] for i in order], 1))
        res = {}
        for n, i in enumerate(order):
            v = lhs[:, 128 * n:128 * n + 128]
            if i == 0:
                v = jnp.concatenate([v, inv[ds(32, 8, c), :]], 0)
            res[i] = _dot(_bf(v), _bf(zz[c // 2][c % 2, ds(64 * i, 64, b), :]))
        part = lambda i, k: res[i][8 * k:8 * k + 8]
        first = sub == 0
        even = [part(0, k) + part(2, k % 8) for k in range(9)]
        for k in range(8):
            sine = part(2, k) if k else jnp.where(first, 0.0, part(2, k))
            odd_t = part(1, k) - part(3, k)
            if k == 7 and c > 0:
                edge = [_unpack(jnp.broadcast_to(us[b, pl.ds(128 * (c - d), 1), :], (8, 128)), 0)
                        for d in (1, 3) if d <= c]
                odd_t = odd_t + kedge[b] * _sum(edge)
            ob[b, pl.ds(128 * c + 64 + 8 * k, 8), :] = _pack(part(0, k) - sine, odd_t)
            ob[b, pl.ds(128 * c + 56 - 8 * k, 8), :] = _pack(
                perm8(jnp.where(first, even[k + 1], even[k]), (8 - sub) & 7), perm8(part(1, k) + part(3, k), rev8))
        if b < 3 and c == NC - 1:
            send(ob.at[b], hu(out_h).at[:, pl.ds(D + 128 * b, 128)])
        if b == 3:
            rows = pl.ds(128 * c, 128)
            send(ob.at[b, rows, :], hu(out_h).at[rows, pl.ds(D + 128 * b, 128)])

    LEFT = ("11", 1, 2, "12", "22", 0, 3)
    RIGHT = ("11", 1, 2, "21", 3, 0, "22")
    X_RIGHT = ("22", 1, 2, "12", 3, 0, "11")
    BLOCKS = ("11", "21", "22", "12")

    def left_sums(a11, a12, a21, a22):
        s1 = a21 + a22
        s2 = s1 - a11
        return [s1, s2, a11 - a21, a12 - s2]

    def right_sums(b11, b12, b21, b22):
        t1 = b12 - b11
        t2 = b22 - t1
        return [t1, t2, b22 - b12, t2 - b21]

    def packed(sums, words):
        lo, hi = [sums(*[_unpack(v, h) for v in words]) for h in range(2)]
        return [_pack(x, y) for x, y in zip(lo, hi)]

    def collect(key, i, m):
        if i == 0:
            held[key] = [m]
        elif i < 3:
            held[key].append(held[key][-1] + m)
        elif i == 3:
            return "11", held[key][0] + m
        elif i == 4:
            return "21", held[key][2] - m
        elif i == 5:
            held[key][1] = held[key][1] + m
            return "22", held[key][2] + m
        else:
            return "12", held.pop(key)[1] + m
        return None, None

    def next_left(key, n, a):
        if n == 0:
            held[key] = a
            return {0: a}
        if n == 1:
            held[key] = held[key], held[key] - a
            return {2: held[key][1]}
        if n == 2:
            a11, s3 = held[key]
            held[key] = a - s3
            return {4: a, 1: held[key], 5: held[key] + a11}
        return {3: a, 6: a - held.pop(key)}

    def next_left_t(key, n, a):
        if n == 0:
            held[key] = a
            return {4: a}
        if n == 1:
            held[key] = held[key], held[key] + a
            return {5: held[key][1]}
        if n == 2:
            a22, s1 = held[key]
            held[key] = s1 - a
            return {0: a, 1: held[key], 2: a22 - held[key]}
        return {3: a, 6: a - held.pop(key)}

    def x_sums(p, kt, r):
        words = [xs[kt + 2 * (e & 1), pl.ds(128 * p + 64 * (e >> 1) + 8 * r, 8), :] for e in range(4)]
        for c, v in enumerate(packed(left_sums, words)):
            xc[p][c, kt, pl.ds(8 * r, 8), :] = v
            if c >= 2:
                pin(v, 10)

    def x_part(which, kt, p, tag):
        if isinstance(which, str):
            return xs[kt + 2 * (int(which[1]) - 1), ds(128 * p + 64 * (int(which[0]) - 1), 64, tag), :]
        return xc[p][which, kt, ds(0, 64, tag), :]

    def wk_sums(cp, r):
        words = [wk[2 * cp + (e & 1), pl.ds(128 * (e >> 1) + 8 * r, 8), :] for e in range(4)]
        for c, v in enumerate(packed(right_sums, words)):
            wkc[cp][c, pl.ds(8 * r, 8), :] = v
            if c >= 2:
                pin(v, 10)

    def wk_part(which, cp, tag):
        if isinstance(which, str):
            return wk[2 * cp + int(which[1]) - 1, ds(128 * (int(which[0]) - 1), 128, tag), :]
        return wkc[cp][which, ds(0, 128, tag), :]

    def feature_map_k(p, cp, name, c):
        for i, v in next_left_t(("pk", cp), BLOCKS.index(name), _phi(c)).items():
            if i >= 5:
                s = v.reshape(16, 8, 128).sum(0)
                held["z", cp, i] = held["z", cp, i] + s if ("z", cp, i) in held else s
            (pk0, pk1)[p // 4][i, cp, p % 4] = settle(_w(v.astype(BF16).T), 64)

    def k_half(p, cp, i):
        def use(m):
            name, c = collect(("kk", cp), i, m)
            if name:
                feature_map_k(p, cp, name, c)
        return [x_part(LEFT[i], kt, p, cp) for kt in range(2)], pinned_rhs(wk_part(RIGHT[i], cp, p)), NN, use

    def k_plain(p, cp, name, h):
        def use(m):
            if h == 0:
                held["half", cp] = m
            else:
                feature_map_k(p, cp, name, held.pop(("half", cp)) + m)
        return ([x_part(name[0] + "12"[h], kt, p, int(name[1]) + 2 * cp) for kt in range(2)],
                pinned_rhs(wk_part("12"[h] + name[1], cp, int(name[0]) + 2 * p)), NN, use)

    def pair(*halves):
        parts = [f() for f in halves]
        lhs = pinned(jnp.concatenate([v for e in parts for v in e[0]], 1))
        for n, (_, rhs, dims, use) in enumerate(parts):
            m = _dot(_bf(lhs[:, 256 * n:256 * n + 256]), _bf(rhs), dims)
            held["last"] = m[:8]
            use(m)

    def g_unit(t, cp, i, j):
        lhs = jnp.concatenate([(pk0, pk1)[t][i, cp, q, ds(0, 64, j), :] for q in range(4)], 1)
        rhs = jnp.concatenate([x_part(X_RIGHT[i], j, 4 * t + q, 4 + cp) for q in range(4)], 0)
        g = _dot(_bf(pinned(lhs)), _bf(pinned_rhs(rhs)))
        held["last"] = g[:8]
        gt = (gt0, gt1)[cp]
        gt[i, j] = g if t == 0 else gt[i, j, ds(0, 128, 0), :] + g

    def put_heads(ref, idx, words):
        for h in range(8):
            ref[(*idx, pl.ds(9 * h, 8), slice(None))] = words[8 * h:8 * h + 8]

    def get_heads(ref, idx, tag):
        return jnp.concatenate([ref[(*idx, pl.ds(zoff[tag % NZ] + r, 8, stride=9), slice(None))] for r in range(8)], 0)

    def wq_parts(cp, kt):
        words = [wq[cp + 2 * (e & 1), pl.ds(128 * (e >> 1) + 64 * kt, 64), :] for e in range(4)]
        sums = packed(right_sums, words)
        for r in range(8):
            for c in (2, 3):
                pin(sums[c][8 * r:8 * r + 8], 11)
        parts = dict(enumerate(sums), **{"11": words[0], "21": words[2], "22": words[3]})
        for i in range(7):
            put_heads(wqt, (i, cp, kt), _w(_bf(parts[RIGHT[i]]).T))

    def z_column(b):
        z = held["z", b // 2, 5] + held["z", b // 2, 6] if b % 2 else held["z", b // 2, 5]
        z = jnp.broadcast_to(z.sum(0, keepdims=True), (8, 128))
        put_heads(zt, (b,), columns(z))
        v = _bf(get_heads(zt, (b,), 0)).astype(F32)
        zb[pl.ds(128 * b, 128), :] = v
        late.append(_w(v[120:]))

    def kv_unit(b):
        row = lax.broadcasted_iota(I32, (128, 128), 0)
        col = lax.broadcasted_iota(I32, (128, 128), 1)
        n = lambda i, j: (gt0, gt1)[b // 2][i, j, ds(0, 128, 1 + b % 2), :]
        if b % 2 == 0:
            both = [n(2, j) - (n(0, j) + n(1, j)) for j in range(2)]
            g = [n(5, j) + both[j] for j in range(2)] + [n(4, j) - both[j] for j in range(2)]
        else:
            g = [n(6, j) + n(5, j) - (n(0, j) + n(1, j)) for j in range(2)] + [n(0, j) + n(3, j) for j in range(2)]
        kv = _dot(jnp.concatenate(g, 1).astype(BF16), _bf(wv[b]))
        put_heads(kvt, (b,), _w(jnp.where((row >> 4) == (col >> 4), kv, 0.0).astype(BF16)))

    def m_unit(b):
        rows = jnp.concatenate([wo[j, pl.ds(64 * b, 64), :] for j in range(4)], 1)
        held["m", b] = _dot(_bf(get_heads(kvt, (b,), 0)), _bf(rows))
        if ("m", b ^ 2) in held:
            for jp in range(2):
                blk = [held["m", b % 2 + 2 * (e >> 1)][:, 128 * (jp + 2 * (e & 1)):128 * (jp + 1 + 2 * (e & 1))]
                       for e in range(4)]
                parts = dict(enumerate(right_sums(*blk)), **{"11": blk[0], "21": blk[2], "22": blk[3]})
                for i in range(7):
                    mm[i, jp, pl.ds(128 * (b % 2), 128), :] = parts[RIGHT[i]].astype(BF16)

    def q_half(p, cp, i):
        def use(m):
            name, c = collect(("q", cp), i, m)
            if not name:
                return
            b = cp + 2 * (int(name[1]) - 1)
            pq = _phi(c)
            rows = [pq[8 * v:8 * v + 8] for v in range(16)]
            scale = []
            for g in range(2):
                s = _sum([rows[v] * zb[ds(128 * b + 8 * v, 8, 2 * p + int(name[0])), :] for v in range(g, 16, 2)])
                den = s + perm8(s, sub ^ 1) + 1e-6
                r = pltpu.reciprocal(den, approx=True)
                scale.append(r * (2.0 - den * r))
            pq = jnp.concatenate([rows[v] * scale[v % 2] for v in range(16)], 0)
            for k, v in next_left(("pq", cp), i - 3, pq).items():
                pqs[p][k, cp] = settle(_w(v.astype(BF16).T), 66)
        return ([get_heads(wqt, (i, cp, kt), p) for kt in range(2)],
                jnp.concatenate([x_part(LEFT[i], kt, p, 8 + cp) for kt in range(2)], 1), NT, use)

    def o_half(p, jp, i):
        def use(m):
            name, c = collect(("o", jp), i, m)
            if name:
                j = jp + 2 * (int(name[1]) - 1)
                block_rows = pl.ds(256 * p + 128 * (int(name[0]) - 1), 128)
                oa[j, block_rows, :] = c.astype(BF16)
                if i in (4, 6) or p == 7:
                    rows = pl.ds(256 * p, 256) if p < 7 else block_rows
                    send(oa.at[j, rows, :], out_h.at[rows, pl.ds(128 * j, 128)])
        return ([pqs[p][i, kt, ds(0, 64, jp), :] for kt in range(2)],
                pinned_rhs(hu(mm)[i, jp, ds(0, 128, p), :]), NN, use)

    plain = [(P(k_plain, p, cp, name, h), [("x", 2 * p + int(name[0]) - 1), ("wk", 2 * cp + int(name[1]) - 1)],
              [("p", h, p, cp)]) for p in range(2) for cp in range(2) for name in BLOCKS for h in range(2)]
    halves = lambda f, kind, ps, c: [(P(f, p, c, i), [], [(kind, i, p, c)]) for p in ps for i in range(7)]
    ahead = halves(k_half, "k", range(2, 8), 0) + halves(q_half, "q", range(8), 0)
    behind = plain[-4:] + halves(k_half, "k", range(2, 8), 1) + halves(q_half, "q", range(8), 1)
    kq = plain[:-4] + [e for both in zip(ahead, behind) for e in both] + behind[len(ahead):]
    os_ = [e for both in zip(*[halves(o_half, "o", range(8), jp) for jp in range(2)]) for e in both]

    def take(src, n):
        out = [(P(pair, src[2 * k][0], src[2 * k + 1][0]), src[2 * k][1] + src[2 * k + 1][1],
                src[2 * k][2] + src[2 * k + 1][2]) for k in range(n)]
        del src[:2 * n]
        return out

    def weave(x, y):
        n = min(len(x), len(y))
        return [e for xy in zip(x, y) for e in xy] + x[n:] + y[n:]

    def with_z(unit, n):
        return lambda: (unit[0](), z_column(2 * n), z_column(2 * n + 1)), unit[1], unit[2] + [("z", 0)]

    gs = [[(P(g_unit, t, cp, i, j), [], [("g", t)]) for cp in range(2) for i in (4, 5, 0, 1, 2, 3, 6)
           for j in range(2)] for t in range(2)]
    kv = lambda b: (P(kv_unit, b), [], [("kv", b % 2)])
    mo = lambda b: (P(m_unit, b), [], [("m", b // 2)])
    attention = take(kq, 35)
    attention += weave(gs[0], take(kq, 25))
    attention += [with_z(gs[1][n], n) for n in range(2)]
    attention += weave(take(kq, 16), gs[1][2:])
    r = take(kq, 10)
    attention += [r[0], r[1], kv(0), r[2], kv(2), r[3], kv(1), r[4], kv(3), mo(0), r[5], mo(2), r[6], mo(1), r[7],
                  mo(3), r[8], r[9]]
    attention += weave(take(os_, len(kq) // 2), take(kq, len(kq) // 2))
    attention += take(os_, len(os_) // 2)

    program = []
    at = {}

    def add(kind, variant, f, *args, needs=()):
        at[(kind, *args)] = len(program)
        program.append((P(f, *args), list(needs), [(kind, variant)]))

    def add_attention(n, needs=()):
        for _ in range(n):
            work, own_needs, parts = attention.pop(0)
            for part in parts:
                at.setdefault(part, len(program))
            program.append((work, own_needs + list(needs), parts))

    count = len(attention)
    add_attention(2)
    for b, end in enumerate((74, 126, 186, count - 5)):
        between, first_u = (22, 2, 0, 0)[b], 0 if b else 12
        for gi in range(16):
            add_attention((between * (gi + 1) + 8) // 16 - (between * gi + 8) // 16)
            for c in range(NC):
                if b > 0 and 2 * c == gi:
                    add("inv", 0, inverse, b - 1, c, needs=["second"])
                if first_u + ((16 - first_u) * (2 * c + 1)) // 16 == gi:
                    add("uhat", 0, uhat, b, c, needs=[("u0", "u1")[c // 4]])
            add("kgen", gi % 2, kgen, b, gi)
        add_attention(2)
        add("tiles", 0, special_tiles, b)
        add_attention(3)
        busy = lambda u: int(any(m == 1 for m, _ in _SLOTS[u]))
        for u in range(3):
            add("khat", busy(u), khat, b, u, needs=["w0"])
        units = end - (count - len(attention))
        for n in range(units):
            for u, mark in enumerate((2, 6, 9, 12, 18), 3):
                if (units * mark * (70 if b == 3 else 100)) // 3200 == n:
                    add("khat", busy(u), khat, b, u, needs=[("w1", "w2", "w2", "x6", "x6")[u - 3]])
            for c in range(NC - 2):
                if b == 3 and units * (22, 25, 28)[c // 2] // 32 == n:
                    add("inv", 0, inverse, 3, c)
            if b == 0 and n == units * 26 // 32:
                at["second"] = len(program)
            add_attention(1, needs=["rest"] if b else ["second"] if "second" in at else [])
    for c in range(NC - 2, NC):
        add("inv", 0, inverse, 3, c)
    add_attention(len(attention))

    size = [dict(kgen=5, tiles=1, inv=4).get(e[2][0][0], 8) for e in program]
    first_row = np.cumsum([0] + size)
    row = lambda *key: first_row[at[key]]

    tails = []

    def factors_job(b, gi):
        mine = []
        if gi < 16:
            others = pins[:]
            del pins[:]
            factors(b, gi)
            mine = pins[:]
            pins[:] = others
        cut = len(mine) * 40 // 100
        keyed = [((i + 0.5) / cut, p) for i, p in enumerate(mine[:cut])]
        keyed += [((i + 0.25) / len(tails), p) for i, p in enumerate(tails)]
        tails[:] = mine[cut:]
        for _, (v, cost, _) in sorted(keyed, key=lambda e: e[0]):
            pin(v, cost)

    jobs = []
    for b in range(4):
        for gi in range(17):
            if b == 0:
                first, needs = (at["p", 0, 0, 1], ("wk", 2)) if gi >= 4 else (0, "first")
            elif b == 1:
                first, needs = max(at["kgen", 0, min(gi, 15)], at["uhat", 0, 4]) + 1, "u1"
            else:
                first, needs = at["kgen", b - 1, min(gi, 15)] + 1, "second"
            jobs.append((first, row("kgen", b, max(gi - 1, 0)) - 4 - (gi == 0),
                         500 * (0.4 if gi == 0 else 0.6 if gi == 16 else 1), [needs], P(factors_job, b, gi)))
        for r in range(8):
            for c in range(0, NC, 2):
                last = row("inv", b, c) if b == 3 else min(row("inv", b, 0), row("uhat", b + 1, 0))
                jobs.append((at["khat", b, (2, 3, 6, 7)[r // 2]] + 2, last - 16, 1210 * (2 * c + 4) / 40, [],
                             P(convolve, r, c)))
    for cp in range(2):
        for r in range(16):
            jobs.append((3 + 3 * cp, row("k", 1, 2, cp) - 14, 20, [("wk", 2 * cp), ("wk", 2 * cp + 1)],
                         P(wk_sums, cp, r)))
    for p in range(8):
        last = row("k", 1, p, 0) - 5 if p >= 2 else row("g", 0) - 14
        first = (14, 14, 18, 27)[p] if p < 4 else at["kgen", 0, 15] if p < 6 else at["khat", 0, 6]
        needs = [("x", 2 * p), ("x", 2 * p + 1)] if p < 4 else ["x4"] if p < 6 else ["x6"]
        for n in range(16):
            jobs.append((first, last - (15 - n) * 10 // 4, 20, needs, P(x_sums, p, n % 2, n // 2)))
    for n in range(4):
        jobs.append((at["second"] + 1, row("q", 0, 0, 0) - 24 - 60 * (3 - n), 176, ["second"],
                     P(wq_parts, n // 2, n % 2)))
    jobs.sort(key=lambda e: e[1])

    own = np.zeros(first_row[-1] + 64)
    for n, unit in enumerate(program):
        for kind, variant, *_ in unit[2]:
            first = first_row[n] + (-8 if kind == "uhat" else size[n] if kind in ("kgen", "inv") else 8)
            own[max(first, 0):first + size[n]] += _LOAD[kind][variant] / (4 * size[n])
    total = np.cumsum(own)

    for n, (work, needs, _) in enumerate(program):
        flush()
        wait(*needs)
        s0, s1 = first_row[n], first_row[n + 1]
        clock[1] = s0
        level, due = 0.0, -credit[0]
        for d, cost in sorted([(e[2], e[1]) for e in pins] + [(e[1], e[2]) for e in jobs]):
            due += cost
            d = max(d, s0 + 1)
            level = max(level, (due + total[d] - total[s0]) / (d - s0))
        share[:] = np.clip(level - own[s0:s1], 0, 70) + (80, 60, 30, 0)[min(n, 3)]
        want = sum(share) + credit[0]
        for job in [e for e in jobs if e[0] <= n]:
            if sum(e[1] for e in pins if e[2] <= job[1]) >= want:
                break
            jobs.remove(job)
            wait(*job[3])
            credit[1] = job[1]
            job[4]()
        assert all(e[1] > s0 for e in jobs)
        if n == at["uhat", 0, 0]:
            skip_table()
        if n == at["uhat", 0, 2]:
            late.extend(held.pop("skip"))
        work()
        clock[0] += 1
    flush(True)
    for c in sent:
        c.wait()
    assert not jobs and not batches and not planned


@jax.jit
def pallas_concat_heads__linear_attn_block__ssm_conv_s4__prompt_kernel(A_x, A_wqkv, A_wo, B_u, B_A_re, B_A_im, B_B_re, B_B_im, B_C_re, B_C_im, B_log_dt, B_Dskip):
    ins = (A_x.reshape(L, D), A_wqkv, A_wo, B_u.reshape(L, D), B_A_re, B_A_im, B_B_re, B_B_im,
           B_C_re, B_C_im, B_log_dt.reshape(4, 128), B_Dskip.reshape(4, 128)) + _constants()
    vm = pltpu.VMEM
    scratch = [
        vm((64, 128), U32), vm((4, L // 2, 128), U32), *[vm((4, D // 2, 128), U32)] * 4,
        vm((4, L // 2, 128), U32), vm((6, D // 2, N), U32), pltpu.SMEM((2, 128), U32),
        vm((256, 128), U32), vm((160, 128), U32), vm((8 * 256, 128), U32),
        vm((7, 2, 2, 72, 128), U32), *[vm((7, 2, 128, 128), F32)] * 2, vm((7, 2, 256, 128), BF16),
        vm((D, 128), F32), vm((4, 72, 128), U32),
        vm((16, 2, 128, 128), U32), vm((3, 128, 128), U32), vm((NC, _U_ROWS, 128), F32),
        vm((4, L // 2, 128), U32), vm((4, L, 128), BF16),
        *[vm((7, 2, 4, 64, 128), U32)] * 2, vm((4, 72, 128), U32), vm((4, 8, 128), F32),
        vm((2, 64, 128), U32), vm((64, 128), U32), vm((4, 64, 128), U32),
        pltpu.SMEM((128,), I32), pltpu.SemaphoreType.DMA((_SEMS,)),
        *[vm((7, 2, 64, 128), U32)] * 8, *[vm((4, 128, 128), U32)] * 2, *[vm((4, 2, 64, 128), U32)] * 8,
        *[vm((NC, _K_ROWS, 128), F32)] * 4, *[vm((64, 128), U32)] * 2, *[vm((2, 256, 128), U32)] * 4,
    ]
    out = pl.pallas_call(
        _kernel,
        out_shape=jax.ShapeDtypeStruct((L, 2 * D), BF16),
        in_specs=[pl.BlockSpec(memory_space=pl.ANY)] * len(ins),
        out_specs=pl.BlockSpec(memory_space=pl.ANY),
        scratch_shapes=scratch,
        compiler_params=pltpu.CompilerParams(vmem_limit_bytes=100 * 2 ** 20,
                                              flags={"XLA_TPU_RESCHEDULE_DMA_DONES": True}),
        name="fused_k",
    )(*ins)
    return out.reshape(1, L, 2 * D)
```

```python
import functools

import jax
import jax.numpy as jnp
import ml_dtypes
import numpy as np
from jax import lax
import jax.experimental.pallas as pl
import jax.experimental.pallas.tpu as pltpu

F32, BF16, U32, I32 = jnp.float32, jnp.bfloat16, jnp.uint32, jnp.int32

L = 2048
D = 512
N = 128
CH = 256
NC = L // CH
NZ = 16
NN = (((1,), (0,)), ((), ()))
NT = (((1,), (1,)), ((), ()))

_OFFSETS = ((0, 2, 4, 6), (1, 3, 5, 7), (256, 258, 260, 262), (512, 516, 768, 772), (1024, 1280, 1536, 1792))
_POWERS = (0, 1, 2, 4, 8, 16, 3, 6, 12, 24, 5, 10, 7, 14, 20, 28, 9, 18, 11, 22, 13, 26, 15, 30,
           17, 19, 21, 23, 25, 27, 29, 31)
_TILES = ((0, 1), (2,), (3,), (3,), (4,), (4,), (4,), (4,))
_ZERO = 24
_SPARE = 32
_SLOTS = (((0, 0), (0, 1), (5, 0), (6, 0)), ((1, 0), (2, 0), (5, 1), (6, 1)), ((3, 0), (4, 0), (7, 0), (7, 1)),
          ((1, 1), (2, 1), (3, 1), (4, 1)), ((0, 2), (0, 3), (5, 2), (6, 2)), ((1, 2), (2, 2), (3, 2), (4, 2)),
          ((7, 2), (7, 3), (5, 3), (6, 3)), ((1, 3), (2, 3), (3, 3), (4, 3)))
_K_IM, _K_ROWS = 72, 144
_U_IM, _U_ROWS = 264, 528
_SEMS = 4

_LOAD = dict(p=(16, 180), k=(16, 32, 32, 136, 168, 216, 192), q=(16, 32, 32, 200, 216, 272, 224),
             o=(16, 32, 32, 40, 40, 56, 40), g=(48, 64), kv=(150, 170), m=(64, 230), z=(60,),
             kgen=(30, 34), uhat=(80,), inv=(75,), khat=(35, 75), tiles=(40,))
_TRIM = [int(c, 16) - 8 for c in (
    "88867998989889988899889999a8745888988886105865788668889866888878899988788756778998989998889999999998"
    "8888999888996689998778888789999999999999888889899889889988898457887789988886676889888899887755899999"
    "8786788788988887888999999998899999998998778778888786688888988877889777786778987867877876888988898878"
    "98889988988998999898989988999999999899989776688886678777786666779999999999999898899999899999999893")]


@functools.cache
def _constants():
    bf = ml_dtypes.bfloat16
    lag = np.arange(L).astype(np.float32).astype(bf).astype(np.int64)
    f = np.concatenate([v for q in range(4) for v in (np.arange(q, 128, 4), 255 - np.arange(q, 128, 4))])
    om = 2 * np.pi * (f + 0.5) / (2 * CH)
    s = np.arange(128) + 0.5
    fwd = np.concatenate([np.cos(om[:, None] * s), -np.sin(om[:, None] * s)], 0)
    low = om.reshape(4, 2, 32)[:, 0].reshape(-1)
    t = np.arange(0, 128, 2)
    inv = np.concatenate([np.cos(low * np.concatenate([t, [128], np.zeros(15)])[:, None]),
                          np.cos(low * (t + 1)[:, None]),
                          np.sin(low * np.where(t, t, 128)[:, None]),
                          np.sin(low * (t + 1)[:, None])], 0) / CH

    def lanes(tile):
        shift = 4 * (tile & 1 if tile < 4 else 0)
        out = np.zeros(128, np.int64)
        for i in range(4):
            for j in range(32):
                out[(32 * (j >> 3) + (j & 7) + 24 + 8 * i + shift) % 128] = _OFFSETS[tile][i] + 8 * _POWERS[j]
        return out

    def spectrum(m, lags):
        phase = np.exp(-1j * om[:, None] * (np.arange(CH)[None, :] - 0.5))
        taps = lambda c: phase @ (lag[CH * c:CH * (c + 1), None] == lags[None, :]).astype(np.float64)
        w = taps(m)
        if m >= 5 or m == 2:
            w = w + 1j * np.where(f % 2, -1, 1)[:, None] * taps(m - 1)
        return np.stack([w.real.reshape(4, 64, -1), w.imag.reshape(4, 64, -1)], 1).reshape(4, 128, 128)

    assert lanes(0)[_ZERO] == 0 and lanes(4)[_ZERO] == 4 * CH and lanes(3)[28] == 2 * CH
    maps = [(m, lanes(tile)) for m in range(NC) for tile in _TILES[m]]
    for m, lags in maps:
        if m in (3, 7):
            assert lags[_SPARE] < CH * m
            lags[_SPARE] = CH * (m + 1)
    mats = [spectrum(m, lags) for m, lags in maps]
    first = lambda q: mats[q % 2].reshape(2, 2, 2, 2, 32, 128)[q // 2, :, :, 0].reshape(128, 128)
    taps = np.concatenate([mats[m + 1][q] if m else first(q) for slots in _SLOTS for m, q in slots], 0)
    return fwd.astype(bf), inv.astype(bf), taps.astype(bf), np.repeat(np.arange(2, dtype=np.int32), NZ)


def _bf(v):
    return pltpu.bitcast(v, BF16)


def _w(v):
    return pltpu.bitcast(v, U32)


def _pack(a, b):
    return pltpu.pack_elementwise([a, b], packed_dtype=BF16)


def _unpack(v, i):
    return pltpu.unpack_elementwise(v, index=i, packed_dtype=BF16, unpacked_dtype=F32)


def _dot(a, b, dims=NN):
    return lax.dot_general(a, b, dims, preferred_element_type=F32)


def _cmul(a, b):
    return a[0] * b[0] - a[1] * b[1], a[0] * b[1] + a[1] * b[0]


def _csq(a):
    t = a[0] * a[1]
    return a[0] * a[0] - a[1] * a[1], t + t


def _phi(t):
    return jnp.where(t > 0, t + 1.0, jnp.exp(t)) + 1e-6


def _sum(xs):
    return functools.reduce(lambda a, b: a + b, xs)


def _kernel(x_h, wqkv_h, wo_h, u_h, are_h, aim_h, bre_h, bim_h, cre_h, cim_h, ldt_h, dsk_h,
            fwd_h, inv_h, taps_h, zero_h, out_h,
            dsk, xs, wq, wk, wv, wo, us, par, ldt, fwd, inv, wm,
            wqt, gt0, gt1, mm, zb, zt, jbuf, kd, uh, ob, oa,
            pk0, pk1, kvt, kedge, kx, k0, dcol, zs, sems, *more):
    pqs, wkc, xc, kh, klast, zz = more[:8], more[8:10], more[10:18], more[18:22], more[22:24], more[24:]
    P = functools.partial
    hu = lambda r: r.bitcast(U32)
    held = {}

    planned, batches, free = {}, {}, list(range(_SEMS))
    late_batches = ("x6", "second", "rest")

    def dma(batch, src, dst):
        planned.setdefault(batch, []).append((src, dst))

    def start():
        while planned and free:
            batch, sem = next(iter(planned)), free.pop(0)
            batches[batch] = sem, [pltpu.make_async_copy(src, dst, sems.at[sem]) for src, dst in planned.pop(batch)]
            for c in batches[batch][1]:
                c.start()

    def wait(*names):
        for n in names:
            assert n not in planned
            if n in batches:
                if n in late_batches:
                    dsk[pl.ds(32 + 8 * late_batches.index(n), 8), :] = _w(held["last"])
                sem, copies = batches.pop(n)
                for c in copies:
                    c.wait()
                free.append(sem)
                start()

    def x_dma(batch, r0, n):
        rows = pl.ds(r0 // 2, n // 2)
        for j in range(4):
            dma(batch, hu(x_h).at[rows, pl.ds(128 * j, 128)], xs.at[j, rows, :])

    def col_dma(batch, src, c0, dst):
        dma(batch, hu(src).at[:, pl.ds(c0, 128)], dst)

    def par_dma(batch, r0, r1):
        for i, r in enumerate((are_h, aim_h, bre_h, bim_h, cre_h, cim_h)):
            dma(batch, hu(r).at[pl.ds(r0, r1 - r0), :], par.at[i, pl.ds(r0, r1 - r0), :])

    def taps_dma(batch, u0, u1):
        rows = pl.ds(256 * u0, 256 * (u1 - u0))
        dma(batch, hu(taps_h).at[rows, :], wm.at[rows, :])

    dma("first", zero_h, zs)
    dma("first", hu(ldt_h), ldt)
    par_dma("first", 0, 16)
    col_dma("first", wqkv_h, D, wk.at[0])
    x_dma("first", 0, 128)
    x_dma(("x", 1), 128, 128)
    col_dma(("wk", 1), wqkv_h, D + 128, wk.at[1])
    par_dma(("wk", 2), 16, 64)
    col_dma(("wk", 2), wqkv_h, D + 256, wk.at[2])
    col_dma(("wk", 3), wqkv_h, D + 384, wk.at[3])
    x_dma(("x", 2), 256, 128)
    x_dma(("x", 3), 384, 128)
    x_dma(("x", 4), 512, 256)
    x_dma(("x", 6), 768, 256)
    dma("u0", hu(fwd_h), fwd)
    dma("u0", hu(dsk_h), dsk.at[pl.ds(0, 2), :])
    for i in range(2):
        dma(("u0", "u1")[i], hu(u_h).at[pl.ds(512 * i, 512), pl.ds(0, 128)], us.at[0, pl.ds(512 * i, 512), :])
    par_dma("u1", 64, 128)
    x_dma("x4", 1024, 512)
    taps_dma("w0", 0, 3)
    taps_dma("w1", 3, 6)
    x_dma("x6", 1536, 512)
    taps_dma("x6", 6, 8)
    dma("second", hu(inv_h), inv.at[pl.ds(0, 136), :])
    col_dma("second", u_h, 128, us.at[1])
    par_dma("second", 128, 256)
    for b in range(4):
        col_dma("second", wqkv_h, 128 * b, wq.at[b])
    for b in range(2, 4):
        col_dma("rest", u_h, 128 * b, us.at[b])
    for b in range(4):
        col_dma("rest", wqkv_h, 2 * D + 128 * b, wv.at[b])
    for b in range(4):
        col_dma("rest", wo_h, 128 * b, wo.at[b])
    start()
    wait("first")

    clock = [0, 0]
    todo, sent = [], []

    def send(src, dst):
        todo.append((clock[0] + 2, src, dst))

    def flush(everything=False):
        while todo and (everything or todo[0][0] <= clock[0]):
            assert not planned and free
            _, src, dst = todo.pop(0)
            sent.append(pltpu.make_async_copy(src, dst, sems.at[free[0]]))
            sent[-1].start()

    zoff = [zs[i] for i in range(NZ)]

    def ds(first, size, tag):
        return pl.ds(pl.multiple_of(zoff[tag % NZ] + first, 8), size)

    sub = lax.broadcasted_iota(I32, (8, 128), 0)
    lane = lax.broadcasted_iota(I32, (8, 128), 1)
    odd = sub & 1
    block = (lane + (104 - 4 * odd)) >> 3
    bit0 = (block & 1) != 0
    bit1 = (block & 2) != 0
    bit0e = (((lane + 104) >> 3) & 1) != 0
    low = sub < 4
    rev8 = 7 - sub
    rev4 = sub ^ 3
    always = [(lane * sub) >= -n for n in range(3)]
    perm8 = lambda v, idx: jnp.take_along_axis(v, idx, axis=0)

    pins = []
    timed = []
    late = []
    share = []
    credit = [0.0, 0]

    def pin(v, cost):
        n = len(pins)
        while n and pins[n - 1][2] > credit[1]:
            n -= 1
        pins.insert(n, (_w(v), cost, credit[1]))

    def settle(words, rows):
        timed.append((clock[1] + rows, _w(words[-8:])))
        timed.sort(key=lambda e: e[0])
        return words

    def pinned(words):
        rows = []
        cols = words.shape[1] // 128
        for i in range(words.shape[0] // 8):
            row = []
            for j in range(cols):
                v = words[8 * i:8 * i + 8, 128 * j:128 * j + 128]
                credit[0] += share[i] / cols
                ties = []
                if timed and timed[0][0] <= clock[1] + i:
                    ties.append(timed.pop(0)[1])
                while pins and credit[0] >= 0.5 * pins[0][1] and len(ties) < (3 if clock[0] < 3 else 1):
                    ties.append(pins[0][0])
                    credit[0] -= pins.pop(0)[1]
                for n, tie in enumerate(ties):
                    v = jnp.where(always[n], v, tie)
                row.append(v)
            rows.append(jnp.concatenate(row, 1))
        if not pins:
            credit[0] = min(credit[0], 0.0)
        return jnp.concatenate(rows, 0)

    def pinned4(tiles):
        v = pinned(jnp.concatenate(tiles, 1))
        return [_bf(v[:, 128 * p:128 * p + 128]) for p in range(4)]

    def pinned_rhs(words):
        if not late:
            return words
        v = [words[8 * i:8 * i + 8] for i in range(words.shape[0] // 8)]
        for j in range(words.shape[0] // 64):
            if late:
                v[8 * j + 7] = jnp.where(always[0], v[8 * j + 7], late.pop(0))
        return jnp.concatenate(v, 0)

    def factors(b, gi):
        un, g = divmod(gi, 2)
        rows = pl.ds(64 * b + 8 * un, 8)
        are, aim, bre, bim, cre, cim = [_unpack(par[i, rows, :], g) for i in range(6)]
        dt = [jnp.full((8, 128), ldt[b // 2, 16 * un + 2 * i + g], U32) for i in range(8)]
        for m in (odd != 0, (sub & 2) != 0, sub >= 4):
            dt = [jnp.where(m, dt[i + 1], dt[i]) for i in range(0, len(dt), 2)]
        pin(dt[0], 15)
        dt = jnp.exp(_unpack(dt[0], b % 2)).astype(BF16).astype(F32)
        pin(dt, 10)
        t = (dt * aim) * np.float32(1.0 / (2.0 * np.pi))
        magic = np.float32(1.5 * 2.0 ** 23)
        x = (t - ((t + magic) - magic)) * np.float32(np.pi / 2.0)
        z = x * x
        pin(z, 9)
        sn = x + x * z * (np.float32(-1.6666654611e-1)
                          + z * (np.float32(8.3321608736e-3) + z * np.float32(-1.9515295891e-4)))
        cs = 1.0 + z * (np.float32(-0.5) + z * (np.float32(4.166664568298827e-2) + z * (
            np.float32(-1.388731625493765e-3) + z * np.float32(2.443315711809948e-5))))
        r = jnp.exp((dt * are) * 0.25)
        a = (r * cs, r * sn)
        pin(cs, 12)
        pin(a[0], 8)
        pin(a[1], 8)
        for i in range(5):
            a = _csq(a)
            if i == 1:
                a1c = (a[0], -a[1])
            if i == 3:
                a4c = (a[0], -a[1])
            if i in (1, 4):
                pin(a[0], 12)
        a8 = (perm8(a[0], rev4), perm8(a[1], rev4))
        made = {0: (jnp.ones_like(dt), jnp.zeros_like(dt)), 1: a8}

        def power(j):
            if j not in made:
                made[j] = _cmul(power(j - 2), power(2)) if j % 2 else _csq(power(j // 2))
            return made[j]

        for k in range(16):
            dst = pl.ds(32 * (k >> 2) + (k & 3), 8, stride=4)
            for c in range(2):
                words = _pack(power(_POWERS[2 * k])[c], power(_POWERS[2 * k + 1])[c])
                jbuf[gi, c, dst, :] = words
            pin(words, 14)
        e = power(32)
        a256c = (perm8(e[0], rev4), -perm8(e[1], rev4))
        quads = [[[None] * 5, [None] * 5], [[None] * 5, [None] * 5]]
        pack = lambda lo, hi: [_pack(lo[c], hi[c]) for c in range(2)]

        def quad(k, p, r, cost):
            for c in range(2):
                r4 = pltpu.roll(r[c], 4, 0)
                quads[0][c][k] = jnp.where(low, p[c], r4)
                quads[1][c][k] = jnp.where(low, r4, p[c])
                pin(quads[0][c][k], cost)

        def times(v, a, anchor=True):
            v = _cmul(v, a)
            if anchor:
                pin(v[0], 9)
            return v

        cb = _cmul((cre, cim), (bre, bim))
        v0 = (cb[0] * dt, -(cb[1] * dt))
        pin(v0[0], 9)
        v4 = times(v0, a4c)
        v256 = times(v0, a256c, False)
        v512 = times(v256, a256c)
        v1 = times(v0, a1c)
        quad(0, pack(v0, v1), pack(v256, v512), 6)
        v260 = times(v4, a256c, False)
        v768 = times(v512, a256c)
        v5 = times(v4, a1c)
        quad(2, pack(v4, v5), pack(v260, v768), 6)
        v1024 = times(v768, a256c)
        v1280 = times(v1024, a256c)
        v1536 = times(v1280, a256c)
        v1792 = times(v1536, a256c, False)
        held["2048", b, gi] = v1792[0] * a256c[0] - v1792[1] * a256c[1]
        if g == 1:
            klast[b % 2][pl.ds(8 * un, 8), :] = _pack(held.pop(("2048", b, gi - 1)), held.pop(("2048", b, gi)))
        quad(4, pack(v1024, v1280), pack(v1536, v1792), 6)
        v516 = times(v260, a256c)
        v2, v6 = times(v1, a1c), times(v5, a1c)
        quad(1, pack(v2, times(v2, a1c, False)), pack(times(v2, a256c, False), v516), 9)
        quad(3, pack(v6, times(v6, a1c, False)), pack(times(v6, a256c, False), times(v516, a256c)), 9)
        held["rows", b, gi] = [jnp.concatenate([jnp.concatenate(quads[q][c], 0) for c in range(2)], 1)
                               for q in range(2)]

    def kgen(b, gi):
        un, g = divmod(gi, 2)
        merged = []
        rows = pinned(jnp.concatenate(held.pop(("rows", b, gi)), 1))
        for q in range(2):
            rhs = jnp.concatenate([
                jnp.concatenate([jbuf[gi, c, pl.ds(32 * jj + 16 * q, 16), :] for jj in range(4)], 0)
                for c in range(2)], 1)
            res = _dot(_bf(rows[:, 256 * q:256 * q + 256]), _bf(rhs), NT)
            held["last"] = res[:8]
            part = lambda i, h: res[16 * i + 8 * (h ^ q):16 * i + 8 * (h ^ q) + 8]
            rot = lambda t, k: pltpu.roll(t, 8 * k, 1, stride=4, stride_axis=0)
            ms = []
            for h in range(2):
                r = [rot(part(k, h), k) for k in range(4)]
                ms.append(jnp.where(bit1, jnp.where(bit0, r[3], r[2]), jnp.where(bit0, r[1], r[0])))
            t = jnp.where(bit1, rot(part(4, 1), 2), rot(part(4, 0), 0))
            ms.append(jnp.where(odd != 0, pltpu.roll(t, 4, 1), t))
            merged.append(ms)
        if g == 0:
            held["taps"] = merged
            return
        for q in range(2):
            for i in range(3):
                kd[i, pl.ds(16 * un + 8 * q, 8), :] = _pack(held["taps"][q][i], merged[q][i])

    def ktile(tile, zero=0):
        load = lambda i, h: jnp.concatenate([kd[i, pl.ds(zero + 16 * un + h, 8, stride=2), :] for un in range(8)], 0)
        if tile < 4:
            return load(tile >> 1, tile & 1)
        return jnp.where(jnp.concatenate([bit0e] * 8, 0), load(2, 1), load(2, 0))

    def columns(row):
        return _w(_bf(jnp.concatenate([_pack(row, row)] * 8, 0)).T)

    def skip_table():
        for b in range(4):
            words = columns(_unpack(jnp.broadcast_to(dsk[pl.ds(b // 2, 1), :], (8, 128)), b % 2))
            dcol[b] = jnp.where(jnp.concatenate([lane == _ZERO] * 8, 0), words, 0)
            held.setdefault("skip", []).append(words[56:])

    def special_tiles(b):
        k0[...] = _pack(*[_unpack(ktile(0), h) + _unpack(dcol[b], h) for h in range(2)])
        spare = jnp.concatenate([lane == _SPARE] * 8, 0)
        rhs = jnp.concatenate([klast[b % 2][ds(0, 64, s), :] for s in range(4)], 0)
        sums = _dot(jnp.ones((16, 128), BF16), _bf(rhs), NT)[0:8]
        sums = [jnp.where(always[0], sums[:, 256 * h:256 * h + 128], sums[:, 256 * h + 128:256 * h + 256])
                for h in range(2)]
        for s, words in enumerate((pltpu.roll(ktile(4), _SPARE - _ZERO, 1), columns(jnp.where(always[1], *sums)))):
            words = jnp.where(spare, words, ktile(3 + s))
            kx[s] = words
            held["tile", (5 + s, 1)] = words[56:]
        row = _unpack(_w(_bf(ktile(3)).T)[8:16], 0)
        kedge[b] = settle(jnp.where(sub == 7, jnp.broadcast_to(row[6:7], (8, 128)), 0.0), 64)

    def khat(b, u):
        lhs = pinned4([wm[ds(256 * u + 64 * i, 64, b), :] for i in range(4)])

        def keep(m, q, re, im):
            if m < 5:
                pr, pi = held.pop(("k", q), (None, None))
                if m < 4:
                    held["k", q] = re, im
                if m > 0:
                    turn = [(re[h] - pi[h], im[h] + pr[h]) if (q + n) % 2 == 0 else (re[h] + pi[h], im[h] - pr[h])
                            for n, h in enumerate((slice(0, 32), slice(32, 64)))]
                    re, im = [jnp.concatenate([e[c] for e in turn], 0) for c in range(2)]
            kh[q][m, pl.ds(0, 64), :] = re
            kh[q][m, pl.ds(_K_IM, 64), :] = im

        for n, (m, q) in enumerate(_SLOTS[u]):
            if m in (3, 7):
                rhs = kx[m // 4, ds(0, 64, q), :]
            elif m == 0 and q % 2 == 0:
                rhs = k0[ds(0, 64, q), :]
            else:
                rhs = ktile(_TILES[m][-1], zoff[4 * (u % 4) + n])
            if ("tile", (m, q)) in held:
                late.append(held.pop(("tile", (m, q))))
                rhs = pinned_rhs(rhs)
            v = _dot(lhs[n], _bf(rhs), NT)
            held["last"] = v[:8]
            if m:
                keep(m, q, v[:64], v[64:])
            elif q % 2 == 0:
                even = v
            else:
                plus, minus = even + v, even - v
                for h in range(2):
                    re, im = slice(64 * h, 64 * h + 32), slice(64 * h + 32, 64 * h + 64)
                    keep(0, q - 1 + h, jnp.concatenate([plus[re], minus[im]], 0),
                         jnp.concatenate([plus[im], minus[re]], 0))

    def uhat(b, c):
        ev, od = [], []
        for k in range(8):
            up = us[b, pl.ds(128 * c + 64 + 8 * k, 8), :]
            down = perm8(us[b, pl.ds(128 * c + 56 - 8 * k, 8), :], rev8)
            u0, u1, d0, d1 = _unpack(up, 0), _unpack(up, 1), _unpack(down, 0), _unpack(down, 1)
            ev.append(_pack(u0 + d1, u1 + d0))
            od.append(_pack(u0 - d1, u1 - d0))
        lhs = pinned4([fwd[ds(64 * p, 64, c), :] for p in range(4)])
        rhs = pinned_rhs(jnp.concatenate(ev, 0)), pinned_rhs(jnp.concatenate(od, 0))
        res = [_dot(lhs[p], _bf(rhs[p // 2])) for p in range(4)]
        held["last"] = res[0][:8]
        for p, v in enumerate(res):
            uh[c, pl.ds(_U_IM * (p // 2) + 128 * (p % 2), 128), :] = v

    def convolve(r, c0):
        q = r // 2
        rest = [0]

        def product(row, whole):
            k = lambda j, o: kh[q][j, ds(_K_IM * o + row, 8, c0), :]
            u = lambda j, o: uh[j, ds(_U_IM * o + 64 * q + row, 8, c0), :]
            acc, cost = {}, {}
            for j in range(c0 + 2):
                for c in range(max(c0, j), c0 + 2):
                    t = _cmul((k(j, 0), k(j, 1)), (u(c - j, 0), u(c - j, 1)))
                    for o in range(2):
                        acc[c, o] = t[o] if j == 0 else acc[c, o] + t[o]
                        cost[c, o] = cost.get((c, o), 0) + (4 if j else 3)
                        if j % 2 and (j < c or whole):
                            pin(acc[c, o], cost.pop((c, o)))
            rest[0] += sum(cost.values())
            return acc

        z = []
        for h in range(2):
            x = product(16 * (r % 2) + 8 * h, True)
            y = product(16 * (r % 2) + 8 * h + 32, h == 0)
            z.append({c: (x[c, 0] + y[c, 0], x[c, 0] - y[c, 0], x[c, 1] - y[c, 1], x[c, 1] + y[c, 1])
                      for c in (c0, c0 + 1)})
        for c in (c0, c0 + 1):
            for i in range(4):
                words = _w(jnp.concatenate([z[0][c][i], z[1][c][i]], 0).astype(BF16))
                zz[c // 2][c % 2, pl.ds(64 * i + 8 * r, 8), :] = words
                pin(words, rest[0] / 8 + 3)

    def inverse(b, c):
        order = [(c + n) % 4 for n in range(4)]
        lhs = pinned(jnp.concatenate([inv[ds((0, 40, 72, 104)[i], 32, c), :] for i in order], 1))
        res = {}
        for n, i in enumerate(order):
            v = lhs[:, 128 * n:128 * n + 128]
            if i == 0:
                v = jnp.concatenate([v, inv[ds(32, 8, c), :]], 0)
            res[i] = _dot(_bf(v), _bf(zz[c // 2][c % 2, ds(64 * i, 64, b), :]))
        part = lambda i, k: res[i][8 * k:8 * k + 8]
        first = sub == 0
        even = [part(0, k) + part(2, k % 8) for k in range(9)]
        for k in range(8):
            sine = part(2, k) if k else jnp.where(first, 0.0, part(2, k))
            odd_t = part(1, k) - part(3, k)
            if k == 7 and c > 0:
                edge = [_unpack(jnp.broadcast_to(us[b, pl.ds(128 * (c - d), 1), :], (8, 128)), 0)
                        for d in (1, 3) if d <= c]
                odd_t = odd_t + kedge[b] * _sum(edge)
            ob[b, pl.ds(128 * c + 64 + 8 * k, 8), :] = _pack(part(0, k) - sine, odd_t)
            ob[b, pl.ds(128 * c + 56 - 8 * k, 8), :] = _pack(
                perm8(jnp.where(first, even[k + 1], even[k]), (8 - sub) & 7), perm8(part(1, k) + part(3, k), rev8))
        if b < 3 and c == NC - 1:
            send(ob.at[b], hu(out_h).at[:, pl.ds(D + 128 * b, 128)])
        if b == 3:
            rows = pl.ds(128 * c, 128)
            send(ob.at[b, rows, :], hu(out_h).at[rows, pl.ds(D + 128 * b, 128)])

    LEFT = ("11", 1, 2, "12", "22", 0, 3)
    RIGHT = ("11", 1, 2, "21", 3, 0, "22")
    X_RIGHT = ("22", 1, 2, "12", 3, 0, "11")
    BLOCKS = ("11", "21", "22", "12")

    def left_sums(a11, a12, a21, a22):
        s1 = a21 + a22
        s2 = s1 - a11
        return [s1, s2, a11 - a21, a12 - s2]

    def right_sums(b11, b12, b21, b22):
        t1 = b12 - b11
        t2 = b22 - t1
        return [t1, t2, b22 - b12, t2 - b21]

    def packed(sums, words):
        lo, hi = [sums(*[_unpack(v, h) for v in words]) for h in range(2)]
        return [_pack(x, y) for x, y in zip(lo, hi)]

    def collect(key, i, m):
        if i == 0:
            held[key] = [m]
        elif i < 3:
            held[key].append(held[key][-1] + m)
        elif i == 3:
            return "11", held[key][0] + m
        elif i == 4:
            return "21", held[key][2] - m
        elif i == 5:
            held[key][1] = held[key][1] + m
            return "22", held[key][2] + m
        else:
            return "12", held.pop(key)[1] + m
        return None, None

    def next_left(key, n, a):
        if n == 0:
            held[key] = a
            return {0: a}
        if n == 1:
            held[key] = held[key], held[key] - a
            return {2: held[key][1]}
        if n == 2:
            a11, s3 = held[key]
            held[key] = a - s3
            return {4: a, 1: held[key], 5: held[key] + a11}
        return {3: a, 6: a - held.pop(key)}

    def next_left_t(key, n, a):
        if n == 0:
            held[key] = a
            return {4: a}
        if n == 1:
            held[key] = held[key], held[key] + a
            return {5: held[key][1]}
        if n == 2:
            a22, s1 = held[key]
            held[key] = s1 - a
            return {0: a, 1: held[key], 2: a22 - held[key]}
        return {3: a, 6: a - held.pop(key)}

    def x_sums(p, kt, r):
        words = [xs[kt + 2 * (e & 1), pl.ds(128 * p + 64 * (e >> 1) + 8 * r, 8), :] for e in range(4)]
        for c, v in enumerate(packed(left_sums, words)):
            xc[p][c, kt, pl.ds(8 * r, 8), :] = v
            if c >= 2:
                pin(v, 10)

    def x_part(which, kt, p, tag):
        if isinstance(which, str):
            return xs[kt + 2 * (int(which[1]) - 1), ds(128 * p + 64 * (int(which[0]) - 1), 64, tag), :]
        return xc[p][which, kt, ds(0, 64, tag), :]

    def wk_sums(cp, r):
        words = [wk[2 * cp + (e & 1), pl.ds(128 * (e >> 1) + 8 * r, 8), :] for e in range(4)]
        for c, v in enumerate(packed(right_sums, words)):
            wkc[cp][c, pl.ds(8 * r, 8), :] = v
            if c >= 2:
                pin(v, 10)

    def wk_part(which, cp, tag):
        if isinstance(which, str):
            return wk[2 * cp + int(which[1]) - 1, ds(128 * (int(which[0]) - 1), 128, tag), :]
        return wkc[cp][which, ds(0, 128, tag), :]

    def feature_map_k(p, cp, name, c):
        for i, v in next_left_t(("pk", cp), BLOCKS.index(name), _phi(c)).items():
            if i >= 5:
                s = v.reshape(16, 8, 128).sum(0)
                held["z", cp, i] = held["z", cp, i] + s if ("z", cp, i) in held else s
            (pk0, pk1)[p // 4][i, cp, p % 4] = settle(_w(v.astype(BF16).T), 64)

    def k_half(p, cp, i):
        def use(m):
            name, c = collect(("kk", cp), i, m)
            if name:
                feature_map_k(p, cp, name, c)
        return [x_part(LEFT[i], kt, p, cp) for kt in range(2)], pinned_rhs(wk_part(RIGHT[i], cp, p)), NN, use

    def k_plain(p, cp, name, h):
        def use(m):
            if h == 0:
                held["half", cp] = m
            else:
                feature_map_k(p, cp, name, held.pop(("half", cp)) + m)
        return ([x_part(name[0] + "12"[h], kt, p, int(name[1]) + 2 * cp) for kt in range(2)],
                pinned_rhs(wk_part("12"[h] + name[1], cp, int(name[0]) + 2 * p)), NN, use)

    def pair(*halves):
        parts = [f() for f in halves]
        lhs = pinned(jnp.concatenate([v for e in parts for v in e[0]], 1))
        for n, (_, rhs, dims, use) in enumerate(parts):
            m = _dot(_bf(lhs[:, 256 * n:256 * n + 256]), _bf(rhs), dims)
            held["last"] = m[:8]
            use(m)

    def g_unit(t, cp, i, j):
        lhs = jnp.concatenate([(pk0, pk1)[t][i, cp, q, ds(0, 64, j), :] for q in range(4)], 1)
        rhs = jnp.concatenate([x_part(X_RIGHT[i], j, 4 * t + q, 4 + cp) for q in range(4)], 0)
        g = _dot(_bf(pinned(lhs)), _bf(pinned_rhs(rhs)))
        held["last"] = g[:8]
        gt = (gt0, gt1)[cp]
        gt[i, j] = g if t == 0 else gt[i, j, ds(0, 128, 0), :] + g

    def put_heads(ref, idx, words):
        for h in range(8):
            ref[(*idx, pl.ds(9 * h, 8), slice(None))] = words[8 * h:8 * h + 8]

    def get_heads(ref, idx, tag):
        return jnp.concatenate([ref[(*idx, pl.ds(zoff[tag % NZ] + r, 8, stride=9), slice(None))] for r in range(8)], 0)

    def wq_parts(cp, kt):
        words = [wq[cp + 2 * (e & 1), pl.ds(128 * (e >> 1) + 64 * kt, 64), :] for e in range(4)]
        sums = packed(right_sums, words)
        for r in range(8):
            for c in (2, 3):
                pin(sums[c][8 * r:8 * r + 8], 11)
        parts = dict(enumerate(sums), **{"11": words[0], "21": words[2], "22": words[3]})
        for i in range(7):
            put_heads(wqt, (i, cp, kt), _w(_bf(parts[RIGHT[i]]).T))

    def z_column(b):
        z = held["z", b // 2, 5] + held["z", b // 2, 6] if b % 2 else held["z", b // 2, 5]
        z = jnp.broadcast_to(z.sum(0, keepdims=True), (8, 128))
        put_heads(zt, (b,), columns(z))
        v = _bf(get_heads(zt, (b,), 0)).astype(F32)
        zb[pl.ds(128 * b, 128), :] = held["zb", b] = v
        late.append(_w(v[120:]))

    def kv_unit(b):
        row = lax.broadcasted_iota(I32, (128, 128), 0)
        col = lax.broadcasted_iota(I32, (128, 128), 1)
        n = lambda i, j: (gt0, gt1)[b // 2][i, j, ds(0, 128, 1 + b % 2), :]
        if b % 2 == 0:
            both = [n(2, j) - (n(0, j) + n(1, j)) for j in range(2)]
            g = [n(5, j) + both[j] for j in range(2)] + [n(4, j) - both[j] for j in range(2)]
        else:
            g = [n(6, j) + n(5, j) - (n(0, j) + n(1, j)) for j in range(2)] + [n(0, j) + n(3, j) for j in range(2)]
        kv = _dot(jnp.concatenate(g, 1).astype(BF16), _bf(wv[b]))
        put_heads(kvt, (b,), _w(jnp.where((row >> 4) == (col >> 4), kv, 0.0).astype(BF16)))

    def m_unit(b):
        rows = jnp.concatenate([wo[j, pl.ds(64 * b, 64), :] for j in range(4)], 1)
        held["m", b] = _dot(_bf(get_heads(kvt, (b,), 0)), _bf(rows))
        if ("m", b ^ 2) in held:
            for jp in range(2):
                blk = [held["m", b % 2 + 2 * (e >> 1)][:, 128 * (jp + 2 * (e & 1)):128 * (jp + 1 + 2 * (e & 1))]
                       for e in range(4)]
                parts = dict(enumerate(right_sums(*blk)), **{"11": blk[0], "21": blk[2], "22": blk[3]})
                for i in range(7):
                    mm[i, jp, pl.ds(128 * (b % 2), 128), :] = parts[RIGHT[i]].astype(BF16)

    def q_half(p, cp, i):
        def use(m):
            name, c = collect(("q", cp), i, m)
            if not name:
                return
            b = cp + 2 * (int(name[1]) - 1)
            assert ("zb", b) in held
            pq = _phi(c)
            rows = [pq[8 * v:8 * v + 8] for v in range(16)]
            scale = []
            for g in range(2):
                s = _sum([rows[v] * zb[ds(128 * b + 8 * v, 8, 2 * p + int(name[0])), :] for v in range(g, 16, 2)])
                den = s + perm8(s, sub ^ 1) + 1e-6
                r = pltpu.reciprocal(den, approx=True)
                scale.append(r * (2.0 - den * r))
            pq = jnp.concatenate([rows[v] * scale[v % 2] for v in range(16)], 0)
            for k, v in next_left(("pq", cp), i - 3, pq).items():
                pqs[p][k, cp] = settle(_w(v.astype(BF16).T), 66)
        return ([get_heads(wqt, (i, cp, kt), p) for kt in range(2)],
                jnp.concatenate([x_part(LEFT[i], kt, p, 8 + cp) for kt in range(2)], 1), NT, use)

    def o_half(p, jp, i):
        def use(m):
            name, c = collect(("o", jp), i, m)
            if name:
                j = jp + 2 * (int(name[1]) - 1)
                block_rows = pl.ds(256 * p + 128 * (int(name[0]) - 1), 128)
                oa[j, block_rows, :] = c.astype(BF16)
                if i in (4, 6) or p == 7:
                    rows = pl.ds(256 * p, 256) if p < 7 else block_rows
                    send(oa.at[j, rows, :], out_h.at[rows, pl.ds(128 * j, 128)])
        return ([pqs[p][i, kt, ds(0, 64, jp), :] for kt in range(2)],
                pinned_rhs(hu(mm)[i, jp, ds(0, 128, p), :]), NN, use)

    plain = [(P(k_plain, p, cp, name, h), [("x", 2 * p + int(name[0]) - 1), ("wk", 2 * cp + int(name[1]) - 1)],
              [("p", h, p, cp)]) for p in range(2) for cp in range(2) for name in BLOCKS for h in range(2)]
    halves = lambda f, kind, ps, c: [(P(f, p, c, i), [], [(kind, i, p, c)]) for p in ps for i in range(7)]
    ahead = halves(k_half, "k", range(2, 8), 0) + halves(q_half, "q", range(8), 0)
    behind = plain[-4:] + halves(k_half, "k", range(2, 8), 1) + halves(q_half, "q", range(8), 1)
    kq = plain[:-4] + [e for both in zip(ahead, behind) for e in both] + behind[len(ahead):]
    n = [e[2][0] for e in kq].index(("q", 3, 0, 0))
    kq[n:n + 4] = [kq[n + i] for i in (3, 1, 0, 2)]
    os_ = [e for both in zip(*[halves(o_half, "o", range(8), jp) for jp in range(2)]) for e in both]

    def take(src, n):
        out = [(P(pair, src[2 * k][0], src[2 * k + 1][0]), src[2 * k][1] + src[2 * k + 1][1],
                src[2 * k][2] + src[2 * k + 1][2]) for k in range(n)]
        del src[:2 * n]
        return out

    def weave(x, y):
        n = min(len(x), len(y))
        return [e for xy in zip(x, y) for e in xy] + x[n:] + y[n:]

    def with_z(unit, n):
        return lambda: (unit[0](), z_column(2 * n), z_column(2 * n + 1)), unit[1], unit[2] + [("z", 0)]

    gs = [[(P(g_unit, t, cp, i, j), [], [("g", t)]) for cp in range(2) for i in (4, 5, 0, 1, 2, 3, 6)
           for j in range(2)] for t in range(2)]
    kv = lambda b: (P(kv_unit, b), [], [("kv", b % 2)])
    mo = lambda b: (P(m_unit, b), [], [("m", b // 2)])
    attention = take(kq, 35)
    attention += weave(gs[0], take(kq, 25))
    attention += [with_z(gs[1][n], n) for n in range(2)]
    attention += weave(take(kq, 16), gs[1][2:])
    r = take(kq, 10)
    attention += [r[0], r[1], kv(0), r[2], kv(2), r[3], kv(1), r[4], kv(3), mo(0), r[5], mo(2), r[6], mo(1), r[7],
                  mo(3), r[8], r[9]]
    attention += weave(take(os_, len(kq) // 2), take(kq, len(kq) // 2))
    attention += take(os_, len(os_) // 2)

    program = []
    at = {}

    def add(kind, variant, f, *args, needs=()):
        at[(kind, *args)] = len(program)
        program.append((P(f, *args), list(needs), [(kind, variant)]))

    def add_attention(n, needs=()):
        for _ in range(n):
            work, own_needs, parts = attention.pop(0)
            for part in parts:
                at.setdefault(part, len(program))
            program.append((work, own_needs + list(needs), parts))

    count = len(attention)
    add_attention(2)
    for b, end in enumerate((74, 126, 186, count - 5)):
        between, first_u = (22, 2, 0, 0)[b], 0 if b else 12
        for gi in range(16):
            add_attention((between * (gi + 1) + 8) // 16 - (between * gi + 8) // 16)
            for c in range(NC):
                if b > 0 and 2 * c == gi:
                    add("inv", 0, inverse, b - 1, c, needs=["second"])
                if first_u + ((16 - first_u) * (2 * c + 1)) // 16 == gi:
                    add("uhat", 0, uhat, b, c, needs=[("u0", "u1")[c // 4]])
            add("kgen", gi % 2, kgen, b, gi)
        add_attention(2)
        add("tiles", 0, special_tiles, b)
        add_attention(3)
        busy = lambda u: int(any(m == 1 for m, _ in _SLOTS[u]))
        for u in range(3):
            add("khat", busy(u), khat, b, u, needs=["w0"])
        units = end - (count - len(attention))
        for n in range(units):
            for u, mark in enumerate((2, 6, 9, 12, 18), 3):
                if (units * mark * (70 if b == 3 else 100)) // 3200 == n:
                    add("khat", busy(u), khat, b, u, needs=["w1" if u < 6 else "x6"])
            for c in range(NC - 2):
                if b == 3 and units * (22, 25, 28)[c // 2] // 32 == n:
                    add("inv", 0, inverse, 3, c)
            if b == 0 and n == units * 26 // 32:
                at["second"] = len(program)
            add_attention(1, needs=["rest"] if b else ["second"] if "second" in at else [])
    for c in range(NC - 2, NC):
        add("inv", 0, inverse, 3, c)
    add_attention(len(attention))

    size = [dict(kgen=5, tiles=1, inv=4).get(e[2][0][0], 8) for e in program]
    first_row = np.cumsum([0] + size)
    row = lambda *key: first_row[at[key]]

    tails = []

    def factors_job(b, gi):
        mine = []
        if gi < 16:
            others = pins[:]
            del pins[:]
            factors(b, gi)
            mine = pins[:]
            pins[:] = others
        cut = len(mine) * 40 // 100
        keyed = [((i + 0.5) / cut, p) for i, p in enumerate(mine[:cut])]
        keyed += [((i + 0.25) / len(tails), p) for i, p in enumerate(tails)]
        tails[:] = mine[cut:]
        for _, (v, cost, _) in sorted(keyed, key=lambda e: e[0]):
            pin(v, cost)

    jobs = []
    for b in range(4):
        for gi in range(17):
            if b == 0:
                first, needs = (at["p", 0, 0, 1], ("wk", 2)) if gi >= 4 else (0, "first")
            elif b == 1:
                first, needs = max(at["kgen", 0, min(gi, 15)], at["uhat", 0, 4]) + 1, "u1"
            else:
                first, needs = at["kgen", b - 1, min(gi, 15)] + 1, "second"
            jobs.append((first, row("kgen", b, max(gi - 1, 0)) - 4 - (gi == 0),
                         500 * (0.4 if gi == 0 else 0.6 if gi == 16 else 1), [needs], P(factors_job, b, gi)))
        for r in range(8):
            for c in range(0, NC, 2):
                last = row("inv", b, c) if b == 3 else min(row("inv", b, 0), row("uhat", b + 1, 0))
                jobs.append((at["khat", b, (2, 3, 6, 7)[r // 2]] + 2, last - 16, 1210 * (2 * c + 4) / 40, [],
                             P(convolve, r, c)))
    for cp in range(2):
        for r in range(16):
            jobs.append((3 + 3 * cp, row("k", 1, 2, cp) - 14, 20, [("wk", 2 * cp), ("wk", 2 * cp + 1)],
                         P(wk_sums, cp, r)))
    for p in range(8):
        last = row("k", 1, p, 0) - 5 if p >= 2 else row("g", 0) - 14
        first = (14, 14, 18, 27)[p] if p < 4 else at["kgen", 0, 15] if p < 6 else at["khat", 0, 6]
        needs = [("x", 2 * p), ("x", 2 * p + 1)] if p < 4 else ["x4"] if p < 6 else ["x6"]
        for n in range(16):
            jobs.append((first, last - (15 - n) * 10 // 4, 20, needs, P(x_sums, p, n % 2, n // 2)))
    for n in range(4):
        jobs.append((at["second"] + 1, row("q", 0, 0, 0) - 24 - 60 * (3 - n), 176, ["second"],
                     P(wq_parts, n // 2, n % 2)))
    jobs.sort(key=lambda e: e[1])

    own = np.zeros(first_row[-1] + 64)
    for n, unit in enumerate(program):
        for kind, variant, *_ in unit[2]:
            first = first_row[n] + (-8 if kind == "uhat" else size[n] if kind in ("kgen", "inv") else 8)
            own[max(first, 0):first + size[n]] += _LOAD[kind][variant] / (4 * size[n])
    total = np.cumsum(own)

    for n, (work, needs, _) in enumerate(program):
        flush()
        wait(*needs)
        s0, s1 = first_row[n], first_row[n + 1]
        clock[1] = s0
        level, due = 0.0, -credit[0]
        for d, cost in sorted([(e[2], e[1]) for e in pins] + [(e[1], e[2]) for e in jobs]):
            due += cost
            d = max(d, s0 + 1)
            level = max(level, (due + total[d] - total[s0]) / (d - s0))
        share[:] = np.clip(level - own[s0:s1] + _TRIM[n], 0, 70) + (80, 60, 30, 0)[min(n, 3)]
        want = sum(share) + credit[0]
        for job in [e for e in jobs if e[0] <= n]:
            if sum(e[1] for e in pins if e[2] <= job[1]) >= want:
                break
            jobs.remove(job)
            wait(*job[3])
            credit[1] = job[1]
            job[4]()
        assert all(e[1] > s0 for e in jobs)
        if n == at["uhat", 0, 0]:
            skip_table()
        if n == at["uhat", 0, 2]:
            late.extend(held.pop("skip"))
        work()
        clock[0] += 1
    flush(True)
    for c in sent:
        c.wait()
    assert not jobs and not batches and not planned


@jax.jit
def pallas_concat_heads__linear_attn_block__ssm_conv_s4__prompt_kernel(A_x, A_wqkv, A_wo, B_u, B_A_re, B_A_im, B_B_re, B_B_im, B_C_re, B_C_im, B_log_dt, B_Dskip):
    ins = (A_x.reshape(L, D), A_wqkv, A_wo, B_u.reshape(L, D), B_A_re, B_A_im, B_B_re, B_B_im,
           B_C_re, B_C_im, B_log_dt.reshape(4, 128), B_Dskip.reshape(4, 128)) + _constants()
    vm = pltpu.VMEM
    scratch = [
        vm((64, 128), U32), vm((4, L // 2, 128), U32), *[vm((4, D // 2, 128), U32)] * 4,
        vm((4, L // 2, 128), U32), vm((6, D // 2, N), U32), pltpu.SMEM((2, 128), U32),
        vm((256, 128), U32), vm((160, 128), U32), vm((8 * 256, 128), U32),
        vm((7, 2, 2, 72, 128), U32), *[vm((7, 2, 128, 128), F32)] * 2, vm((7, 2, 256, 128), BF16),
        vm((D, 128), F32), vm((4, 72, 128), U32),
        vm((16, 2, 128, 128), U32), vm((3, 128, 128), U32), vm((NC, _U_ROWS, 128), F32),
        vm((4, L // 2, 128), U32), vm((4, L, 128), BF16),
        *[vm((7, 2, 4, 64, 128), U32)] * 2, vm((4, 72, 128), U32), vm((4, 8, 128), F32),
        vm((2, 64, 128), U32), vm((64, 128), U32), vm((4, 64, 128), U32),
        pltpu.SMEM((2 * NZ,), I32), pltpu.SemaphoreType.DMA((_SEMS,)),
        *[vm((7, 2, 64, 128), U32)] * 8, *[vm((4, 128, 128), U32)] * 2, *[vm((4, 2, 64, 128), U32)] * 8,
        *[vm((NC, _K_ROWS, 128), F32)] * 4, *[vm((64, 128), U32)] * 2, *[vm((2, 256, 128), U32)] * 4,
    ]
    out = pl.pallas_call(
        _kernel,
        out_shape=jax.ShapeDtypeStruct((L, 2 * D), BF16),
        in_specs=[pl.BlockSpec(memory_space=pl.ANY)] * len(ins),
        out_specs=pl.BlockSpec(memory_space=pl.ANY),
        scratch_shapes=scratch,
        compiler_params=pltpu.CompilerParams(vmem_limit_bytes=100 * 2 ** 20,
                                              flags={"XLA_TPU_RESCHEDULE_DMA_DONES": True}),
        name="fused_k",
    )(*ins)
    return out.reshape(1, L, 2 * D)
```
